```python
import os as _os
_os.environ.setdefault("JAX_PLATFORMS", "cpu")
import jax
import jax.numpy as jnp

def _softmax(x, axis=-1):
    return jax.nn.softmax(x, axis=axis)
def _gelu(x):
    return jax.nn.gelu(x, approximate=True)
def _silu(x):
    return jax.nn.silu(x)
def _sigmoid(x):
    return jax.nn.sigmoid(x)
def _layernorm(x, axis=-1, eps=1e-5):
    m = jnp.mean(x, axis=axis, keepdims=True)
    v = jnp.var(x, axis=axis, keepdims=True)
    return (x - m) / jnp.sqrt(v + eps)
def _scatter_add(tgt, idx, src, axis=0):
    return tgt.at[idx].add(src)
def _segment_sum(src, seg, n):
    return jax.ops.segment_sum(src, seg, n)
class _Rng:
    def __init__(self, key):
        self._k = key
    def _next(self):
        self._k, sub = jax.random.split(self._k)
        return sub
    def normal(self, shape):
        return jax.random.normal(self._next(), shape, dtype=jnp.bfloat16)
    def randint(self, lo, hi, shape):
        return jax.random.randint(self._next(), shape, lo, hi, dtype=jnp.int32)
    def uniform(self, shape, lo=0.0, hi=1.0):
        return jax.random.uniform(self._next(), shape, jnp.bfloat16, lo, hi)
    def permutation(self, n):
        return jax.random.permutation(self._next(), n)


kernel_name = 'interleave_layers__linear_attn_block__mha_block__prompt'

def setup_inputs():
    _rng = _Rng(jax.random.key(int.from_bytes(__import__("os").urandom(4), "little")))
    _w = (lambda a: (lambda t: t.astype(jnp.bfloat16) if jnp.issubdtype(t.dtype, jnp.floating) else t)(jnp.asarray(a)))
    def _A_setup():
        B, S, D = 1, 2048, 640
        return {
            "x": _w((lambda *s: _rng.normal(s) * 0.05)(B, S, D)),
            "wqkv": _w((lambda *s: _rng.normal(s) * 0.1)(D, 3 * D)),
            "wo": _w((lambda *s: _rng.normal(s) * 0.05)(D, D)),
        }
    _A_in = _A_setup()

    def _B_setup():
        B, S, D, H = 1, 2048, 640, 32
        return {
            "x": _w((lambda *s: _rng.normal(s) * 0.05)(B, S, D)),
            "wqkv": _w((lambda *s: _rng.normal(s) * 0.1)(D, 3 * D)),
            "wo": _w((lambda *s: _rng.normal(s) * 0.05)(D, D)),
        }
    _B_in = _B_setup()

    return {
        "A_x": _A_in["x"],
        "A_wqkv": _A_in["wqkv"],
        "A_wo": _A_in["wo"],
        "B_x": _B_in["x"],
        "B_wqkv": _B_in["wqkv"],
        "B_wo": _B_in["wo"],
    }

def reference(A_x, A_wqkv, A_wo, B_x, B_wqkv, B_wo):
    def _A_ref(x, wqkv, wo):
        B, S, D = x.shape
        H = 32; Dh = D // H
        qkv = (lambda x, *d: x.transpose(*d))((x @ wqkv).reshape(B, S, 3, H, Dh), 2, 0, 3, 1, 4)
        q, k, v = qkv[0], qkv[1], qkv[2]
        phi = lambda t: jnp.where(t > 0, t + 1, jnp.exp(t)) + 1e-6
        pq, pk = phi(q), phi(k)
        kv = jnp.einsum("bhsd,bhse->bhde", pk, v)
        z = jnp.einsum("bhsd->bhd", pk)
        num = jnp.einsum("bhqd,bhde->bhqe", pq, kv)
        den = jnp.einsum("bhqd,bhd->bhq", pq, z)[..., None] + 1e-6
        o = num / den
        return (lambda x, *d: x.transpose(*d))(o, 0, 2, 1, 3).reshape(B, S, D) @ wo

    def _B_ref(x, wqkv, wo):
        B, S, D = x.shape
        H = 32
        Dh = D // H
        qkv = (lambda x, *d: x.transpose(*d))((x @ wqkv).reshape(B, S, 3, H, Dh), 2, 0, 3, 1, 4)
        q, k, v = qkv[0], qkv[1], qkv[2]
        scores = jnp.einsum("bhqd,bhkd->bhqk", q, k) * (Dh ** -0.5)
        p = _softmax(scores, axis=-1)
        o = jnp.einsum("bhqk,bhkd->bhqd", p, v)
        return (lambda x, *d: x.transpose(*d))(o, 0, 2, 1, 3).reshape(B, S, D) @ wo

    x = A_x
    x = x + _A_ref(_layernorm(x, axis=-1), A_wqkv, A_wo)
    x = x + _B_ref(_layernorm(x, axis=-1), B_wqkv, B_wo)
    x = x + _A_ref(_layernorm(x, axis=-1), A_wqkv, A_wo)
    x = x + _B_ref(_layernorm(x, axis=-1), B_wqkv, B_wo)
    return x
```

```python
import functools
import math

import jax
import jax.numpy as jnp
import jax.experimental.pallas as pl
import jax.experimental.pallas.tpu as pltpu

S = 2048
D = 640
H = 32
DH = 20
LANES = 128
NDT = D // LANES
RB = 512
NRB = S // RB
TQ = 512
NQB = S // TQ
KC = 128
VR = 24
EPS = 1e-5

STRADDLE = tuple(h for h in range(H) if (h * DH) // LANES != (h * DH + DH - 1) // LANES)
assert len(STRADDLE) * DH <= LANES

NT = (((1,), (1,)), ((), ()))

BF16 = jnp.bfloat16
F32 = jnp.float32


def _phi(t):
    return jnp.where(t > 0, t + 1.0, jnp.exp(t)) + 1e-6


def _layernorm(x):
    m = jnp.mean(x, axis=-1, keepdims=True)
    xc = x - m
    v = jnp.mean(xc * xc, axis=-1, keepdims=True)
    return xc * jax.lax.rsqrt(v + EPS)


def _kv_windows():
    wins = []
    for j in range(NDT):
        h0 = (j * LANES) // DH
        h1 = (j * LANES + LANES - 1) // DH
        lo = (h0 * DH) // 16 * 16
        hi = -(-((h1 + 1) * DH) // 16) * 16
        wins.append((lo, hi))
    return wins


def _kernel(x_ref, a_wqkv_ref, a_wkt_ref, a_wo_ref, b_wqkv_ref, b_wqx_ref, b_wkx_ref,
            b_wvt_ref, b_wo_ref, o_ref,
            x_scr, xn_scr, pq_scr, kv_scr, z_scr, m_scr_w, z32_scr,
            q_scr, k_scr, vt_scr, s_scr, mx_scr, ot_scr):
    wins = _kv_windows()

    def rows(i):
        return pl.ds(pl.multiple_of(i * RB, RB), RB)

    def init_body(i, c):
        x = x_ref[rows(i), :].astype(F32)
        x_scr[rows(i), :] = x
        xn_scr[rows(i), :] = _layernorm(x).astype(BF16)
        return c

    jax.lax.fori_loop(0, NRB, init_body, 0)

    def residual_update(i, out, last):
        x = x_scr[rows(i), :] + out
        if last:
            o_ref[rows(i), :] = x.astype(o_ref.dtype)
        else:
            x_scr[rows(i), :] = x
            xn_scr[rows(i), :] = _layernorm(x).astype(BF16)

    def layer_a():
        kv_scr[...] = jnp.zeros_like(kv_scr)
        z_scr[...] = jnp.zeros_like(z_scr)

        def proj_body(i, c):
            xn = xn_scr[rows(i), :]
            q = jnp.dot(xn, a_wqkv_ref[:, 0:D], preferred_element_type=F32)
            pq_scr[rows(i), :] = _phi(q).astype(BF16)
            v = jnp.dot(xn, a_wqkv_ref[:, 2 * D:3 * D], preferred_element_type=F32).astype(BF16)
            kt = jax.lax.dot_general(a_wkt_ref[...], xn, NT, preferred_element_type=F32)
            pkt = _phi(kt)
            zacc = pkt[:, 0:LANES]
            for t in range(1, RB // LANES):
                zacc = zacc + pkt[:, t * LANES:(t + 1) * LANES]
            z_scr[...] += zacc
            pkt = pkt.astype(BF16)
            for j, (lo, hi) in enumerate(wins):
                kv_scr[lo:hi, j * LANES:(j + 1) * LANES] += jnp.dot(
                    pkt[lo:hi, :], v[:, j * LANES:(j + 1) * LANES], preferred_element_type=F32)
            return c

        jax.lax.fori_loop(0, NRB, proj_body, 0)

        rh = jax.lax.broadcasted_iota(jnp.int32, (D, D), 0) // DH
        ch = jax.lax.broadcasted_iota(jnp.int32, (D, D), 1) // DH
        kv_bd = jnp.where(rh == ch, kv_scr[...], 0.0).astype(BF16)
        m_scr_w[...] = jnp.dot(kv_bd, a_wo_ref[...], preferred_element_type=F32).astype(BF16)
        z = jnp.sum(z_scr[...], axis=1, keepdims=True)
        rh2 = jax.lax.broadcasted_iota(jnp.int32, (D, LANES), 0) // DH
        c2 = jax.lax.broadcasted_iota(jnp.int32, (D, LANES), 1)
        sel = (c2 < 2 * H) & (rh2 == c2 % H)
        z32_scr[...] = jnp.where(sel, z, 0.0).astype(BF16)

        er = jax.lax.broadcasted_iota(jnp.int32, (LANES, D), 0)
        ec = jax.lax.broadcasted_iota(jnp.int32, (LANES, D), 1) // DH
        e2 = jnp.where((er < 2 * H) & (ec == er % H), 1.0, 0.0).astype(BF16)

        def out_body(i, c):
            pq = pq_scr[rows(i), :]
            den = jnp.dot(pq, z32_scr[...], preferred_element_type=F32) + 1e-6
            r = 1.0 / den
            r_hi = r.astype(BF16).astype(F32)
            lane = jax.lax.broadcasted_iota(jnp.int32, r.shape, 1)
            rin = jnp.where(lane < H, r_hi, r - r_hi).astype(BF16)
            r_exp = jnp.dot(rin, e2, preferred_element_type=F32)
            y = (pq.astype(F32) * r_exp).astype(BF16)
            out = jnp.dot(y, m_scr_w[...], preferred_element_type=F32)
            residual_update(i, out, False)
            return c

        jax.lax.fori_loop(0, NRB, out_body, 0)

    qscale = (DH ** -0.5) * math.log2(math.e)

    def head_loc(h):
        g = (h * DH) // LANES
        off = (h * DH) % LANES
        for n, hs in enumerate(STRADDLE):
            g = jnp.where(h == hs, NDT, g)
            off = jnp.where(h == hs, n * DH, off)
        return g, off

    def layer_b(last):
        def proj_body(i, c):
            xn = xn_scr[rows(i), :]
            q = jnp.dot(xn, b_wqkv_ref[:, 0:D], preferred_element_type=F32) * qscale
            for g in range(NDT):
                q_scr[g, rows(i), :] = q[:, g * LANES:(g + 1) * LANES].astype(BF16)
            qx = jnp.dot(xn, b_wqx_ref[...], preferred_element_type=F32) * qscale
            q_scr[NDT, rows(i), :] = qx.astype(BF16)
            k = jnp.dot(xn, b_wqkv_ref[:, D:2 * D], preferred_element_type=F32)
            for g in range(NDT):
                k_scr[g, rows(i), :] = k[:, g * LANES:(g + 1) * LANES].astype(BF16)
            kx = jnp.dot(xn, b_wkx_ref[...], preferred_element_type=F32)
            k_scr[NDT, rows(i), :] = kx.astype(BF16)
            vt = jax.lax.dot_general(b_wvt_ref[...], xn, NT, preferred_element_type=F32)
            sub = jax.lax.broadcasted_iota(jnp.int32, (8, RB), 0)
            for p in range(H // 2):
                b = p * 2 * DH
                mid = vt[b + 16:b + 24, :]
                vt_scr[p * 2 * VR:p * 2 * VR + 16, rows(i)] = vt[b:b + 16, :]
                vt_scr[p * 2 * VR + 16:p * 2 * VR + 24, rows(i)] = jnp.where(sub < 4, mid, 1.0)
                vt_scr[p * 2 * VR + 24:p * 2 * VR + 32, rows(i)] = jnp.where(sub < 4, 1.0, mid)
                vt_scr[p * 2 * VR + 32:p * 2 * VR + 48, rows(i)] = vt[b + 24:b + 40, :]
            return c

        jax.lax.fori_loop(0, NRB, proj_body, 0)

        n_stage = NQB * H

        def stage(i_qk, slot_qk, i_pv, slot_pv):
            h = i_qk % H
            qb = i_qk // H
            g, off = head_loc(h)
            q = q_scr[g, pl.ds(pl.multiple_of(qb * TQ, TQ), TQ), :]
            lane = jax.lax.broadcasted_iota(jnp.int32, (TQ, LANES), 1)
            qm = jnp.where((lane >= off) & (lane < off + DH), q, jnp.zeros_like(q))
            if i_pv is not None:
                hp = i_pv % H
                mprev = mx_scr[slot_pv]
                vrows = pl.ds(pl.multiple_of(hp * VR, 8), VR)
            mx = None
            o = None
            for c in range(S // KC):
                ks = slice(c * KC, (c + 1) * KC)
                s = jax.lax.dot_general(k_scr[g, ks, :], qm, NT, preferred_element_type=F32)
                s_scr[slot_qk, ks, :] = s
                cm = jnp.max(s.reshape(KC // 8, 8, TQ), axis=0)
                mx = cm if mx is None else jnp.maximum(mx, cm)
                if i_pv is not None:
                    p = jnp.exp2(s_scr[slot_pv, ks, :] - mprev).astype(BF16)
                    oc = jnp.dot(vt_scr[vrows, ks], p, preferred_element_type=F32)
                    o = oc if o is None else o + oc
            mx_scr[slot_qk] = jnp.max(mx, axis=0, keepdims=True)
            return o

        stage(0, 0, None, None)

        def attn_body(j, c):
            i = 2 * j
            o_even = stage(i + 1, 1, i, 0)
            o_odd = stage(jnp.minimum(i + 2, n_stage - 1), 0, i + 1, 1)
            o_even = o_even * (1.0 / o_even[DH:DH + 1, :])
            o_odd = o_odd * (1.0 / o_odd[0:1, :])
            sub = jax.lax.broadcasted_iota(jnp.int32, (8, TQ), 0)
            mid = jnp.where(sub < 4, o_even[16:24, :], o_odd[0:8, :])
            pair = jnp.concatenate([o_even[0:16, :], mid, o_odd[8:24, :]], axis=0)
            p = j % (H // 2)
            qb = j // (H // 2)
            ot_scr[pl.ds(pl.multiple_of(p * 2 * DH, 8), 2 * DH),
                   pl.ds(pl.multiple_of(qb * TQ, TQ), TQ)] = pair
            return c

        jax.lax.fori_loop(0, n_stage // 2, attn_body, 0)

        def out_body(i, c):
            o = ot_scr[:, rows(i)].T.astype(BF16)
            out = jnp.dot(o, b_wo_ref[...], preferred_element_type=F32)
            residual_update(i, out, last)
            return c

        jax.lax.fori_loop(0, NRB, out_body, 0)

    layer_a()
    layer_b(False)
    layer_a()
    layer_b(True)


@jax.jit
def pallas_interleave_layers__linear_attn_block__mha_block__prompt_kernel(
    A_x: jax.Array,
    A_wqkv: jax.Array,
    A_wo: jax.Array,
    B_x: jax.Array,
    B_wqkv: jax.Array,
    B_wo: jax.Array,
):
    del B_x
    x = A_x.reshape(S, D)
    a_wkt = A_wqkv[:, D:2 * D].T
    b_wvt = B_wqkv[:, 2 * D:3 * D].T

    def extra(base):
        cols = [B_wqkv[:, base + h * DH:base + (h + 1) * DH] for h in STRADDLE]
        w = jnp.concatenate(cols, axis=1)
        return jnp.pad(w, ((0, 0), (0, LANES - len(STRADDLE) * DH)))

    b_wqx = extra(0)
    b_wkx = extra(D)

    scratch = [
        pltpu.VMEM((S, D), F32),
        pltpu.VMEM((S, D), BF16),
        pltpu.VMEM((S, D), BF16),
        pltpu.VMEM((D, D), F32),
        pltpu.VMEM((D, LANES), F32),
        pltpu.VMEM((D, D), BF16),
        pltpu.VMEM((D, LANES), BF16),
        pltpu.VMEM((NDT + 1, S, LANES), BF16),
        pltpu.VMEM((NDT + 1, S, LANES), BF16),
        pltpu.VMEM((H * VR, S), F32),
        pltpu.VMEM((2, S, TQ), F32),
        pltpu.VMEM((2, 1, TQ), F32),
        pltpu.VMEM((D, S), F32),
    ]
    out = pl.pallas_call(
        _kernel,
        out_shape=jax.ShapeDtypeStruct((S, D), A_x.dtype),
        scratch_shapes=scratch,
        compiler_params=pltpu.CompilerParams(vmem_limit_bytes=100 * 1024 * 1024),
    )(x, A_wqkv, a_wkt, A_wo, B_wqkv, b_wqx, b_wkx, b_wvt, B_wo)
    return out.reshape(1, S, D)
```

```python
import math

import jax
import jax.numpy as jnp
import jax.experimental.pallas as pl
import jax.experimental.pallas.tpu as pltpu

S = 2048
D = 640
H = 32
DH = 20
LANES = 128
NDT = D // LANES
RB = 512
HB = 256
NRB = S // RB
TQ = 512
NQB = S // TQ
KC = 512
PKC = 128
NS = 2
W = TQ // NS
NC = S // KC
VR = 24
UNROLL = 8
EPS = 1e-5

NT = (((1,), (1,)), ((), ()))

BF16 = jnp.bfloat16
F32 = jnp.float32
U32 = jnp.uint32
I32 = jnp.int32
I8 = jnp.int8

RND = 12582912.0


def _phi(t):
    return jnp.where(t > 0, t + 1.0, jnp.exp(t)) + 1e-6


def _layernorm(x):
    m = jnp.mean(x, axis=-1, keepdims=True)
    xc = x - m
    v = jnp.mean(xc * xc, axis=-1, keepdims=True)
    return xc * jax.lax.rsqrt(v + EPS)


def _kv_windows():
    wins = []
    for j in range(NDT):
        h0 = (j * LANES) // DH
        h1 = (j * LANES + LANES - 1) // DH
        lo = (h0 * DH) // 16 * 16
        hi = -(-((h1 + 1) * DH) // 16) * 16
        wins.append((lo, hi))
    return wins


WINS = _kv_windows()


def _iota(shape, dim):
    return jax.lax.broadcasted_iota(jnp.int32, shape, dim)


def _pack8(y):
    return pltpu.bitcast(pltpu.bitcast(y, I32).astype(I8), U32)


def _limbs(t):
    ya = t + RND
    frac = t - (ya - RND)
    return ya, t * 0.125 + RND, frac * 16.0 + RND


def _kernel(x_hbm, awqkv_hbm, awo_hbm, bwqkv_hbm, bwo_hbm, o_hbm,
            xio, awqkv, awo, bwqkv, bwo, awkt, bwqvt,
            x_scr, pq_scr, y_scr, g_scr, z_scr, mw_scr, zt_scr,
            xn_scr, kf_scr, kmax_scr, kinv_scr, ksc_scr,
            qw_scr, mg_scr, k8_scr, vt_scr, s_scr, mx_scr, oacc_scr, ot_scr,
            xsem, wsem, osem):

    def blk(i):
        return pl.ds(pl.multiple_of(i * RB, RB), RB)

    def half(i, t):
        return pl.ds(pl.multiple_of(i * RB + t * HB, HB), HB)

    def x_copy(i):
        return pltpu.make_async_copy(x_hbm.at[blk(i), :], xio.at[blk(i), :], xsem.at[i])

    def o_copy(i):
        return pltpu.make_async_copy(xio.at[blk(i), :], o_hbm.at[blk(i), :], osem.at[i])

    cp_awk = pltpu.make_async_copy(awqkv_hbm.at[:, D:2 * D], awqkv.at[:, D:2 * D], wsem.at[0])
    cp_awq = pltpu.make_async_copy(awqkv_hbm.at[:, 0:D], awqkv.at[:, 0:D], wsem.at[1])
    cp_awv = pltpu.make_async_copy(awqkv_hbm.at[:, 2 * D:3 * D], awqkv.at[:, 2 * D:3 * D], wsem.at[2])
    cp_awo = pltpu.make_async_copy(awo_hbm, awo, wsem.at[3])
    cp_bwqkv = pltpu.make_async_copy(bwqkv_hbm, bwqkv, wsem.at[4])
    cp_bwo = pltpu.make_async_copy(bwo_hbm, bwo, wsem.at[5])

    def a_zero():
        g_scr[...] = jnp.zeros_like(g_scr)
        z_scr[...] = jnp.zeros_like(z_scr)

    def a_proj(i, xns):
        pkts = []
        for t, xn in enumerate(xns):
            kt = jax.lax.dot_general(awkt[...], xn, NT, preferred_element_type=F32)
            pkts.append(_phi(kt))
        for t, xn in enumerate(xns):
            q = jnp.dot(xn, awqkv[:, 0:D], preferred_element_type=F32)
            pq_scr[half(i, t), :] = _phi(q).astype(BF16)
        pkt = jnp.concatenate(pkts, axis=1)
        zacc = pkt[:, 0:LANES]
        for t in range(1, RB // LANES):
            zacc = zacc + pkt[:, t * LANES:(t + 1) * LANES]
        z_scr[...] += zacc
        g_scr[...] += jnp.dot(pkt.astype(BF16), jnp.concatenate(xns, axis=0),
                              preferred_element_type=F32)

    def a_norm(i):
        for t in range(RB // HB):
            pq = pq_scr[half(i, t), :]
            den = jnp.dot(pq, zt_scr[...], preferred_element_type=F32) + 1e-6
            r = 1.0 / den
            r_exp = jnp.concatenate(
                [jnp.take_along_axis(r, (_iota((HB, LANES), 1) + j * LANES) // DH, axis=1)
                 for j in range(NDT)], axis=1)
            y_scr[half(i, t), :] = (pq.astype(F32) * r_exp).astype(BF16)

    def a_mid():
        z = jnp.sum(z_scr[...], axis=1, keepdims=True)
        rh = _iota((D, LANES), 0) // DH
        zt_scr[...] = jnp.where(rh == _iota((D, LANES), 1), z, 0.0).astype(BF16)
        a_norm(0)
        g = g_scr[...].astype(BF16)
        parts = []
        for j, (lo, hi) in enumerate(WINS):
            n = hi - lo
            kvj = jnp.dot(g[lo:hi, :], awqkv[:, 2 * D + j * LANES:2 * D + (j + 1) * LANES],
                          preferred_element_type=F32)
            rh = (_iota((n, LANES), 0) + lo) // DH
            ch = (_iota((n, LANES), 1) + j * LANES) // DH
            kvj = jnp.where(rh == ch, kvj, 0.0).astype(BF16)
            parts.append(jnp.dot(kvj, awo[j * LANES:(j + 1) * LANES, :], preferred_element_type=F32))
        for j, (lo, hi) in enumerate(WINS):
            s0 = lo if j == 0 else WINS[j - 1][1]
            s1 = hi if j == NDT - 1 else WINS[j + 1][0]
            mw_scr[s0:s1, :] = parts[j][s0 - lo:s1 - lo, :].astype(BF16)
            if j < NDT - 1:
                mw_scr[s1:hi, :] = (parts[j][s1 - lo:hi - lo, :]
                                    + parts[j + 1][0:hi - s1, :]).astype(BF16)
        kmax_scr[...] = jnp.zeros_like(kmax_scr)

    def a_out(i, t):
        return jnp.dot(y_scr[half(i, t), :], mw_scr[...], preferred_element_type=F32)

    qscale = (DH ** -0.5) * math.log2(math.e)

    def b_proj_k(i, t, xn):
        k = jnp.dot(xn, bwqkv[:, D:2 * D], preferred_element_type=F32)
        kf_scr[half(i, t), :] = k
        kmax_scr[...] = jnp.maximum(kmax_scr[...],
                                    jnp.max(jnp.abs(k).reshape(HB // 8, 8, D), axis=0))

    def b_mid():
        kmax = jnp.max(kmax_scr[...], axis=0, keepdims=True)
        kmax = jnp.maximum(kmax, 1e-30)
        kinv_scr[...] = jnp.broadcast_to(127.0 / kmax, (8, D))
        ksc_scr[...] = jnp.broadcast_to(kmax * (qscale / 127.0), (LANES, D)).T

    def b_proj_qv(i, t):
        cols = half(i, t)
        xn = xn_scr[cols, :]
        qvt = jax.lax.dot_general(bwqvt[...], xn, NT, preferred_element_type=F32)
        row = _iota((VR, HB), 0)
        zero8 = jnp.full((8, HB), RND, F32)
        for h in range(H):
            off = (h * DH) % 8
            w0 = h * DH - off
            ksc = jnp.concatenate([ksc_scr[w0:w0 + VR, :]] * (HB // LANES), axis=1)
            q = jnp.where((row >= off) & (row < off + DH), qvt[w0:w0 + VR, :] * ksc, 0.0)
            qmax = jnp.max(jnp.abs(q), axis=0, keepdims=True) * (1.0 / 127.0)
            eb = jnp.clip(pltpu.bitcast(qmax, I32) >> 23, 66, 226)
            qt = q * pltpu.bitcast((253 - eb) << 23, F32)
            ya, y8, yf = _limbs(qt)
            pa = _pack8(jnp.concatenate([ya, zero8], axis=0))
            qw_scr[h, 0:8, cols] = pa
            qw_scr[h, 8:16, cols] = pa
            qw_scr[h, 16:24, cols] = _pack8(jnp.concatenate([y8, zero8], axis=0))
            qw_scr[h, 24:32, cols] = _pack8(jnp.concatenate([yf, zero8], axis=0))
            mg_scr[h, :, cols] = jnp.broadcast_to(((eb + 23) << 23) | 0x400000, (8, HB))
        sub = _iota((8, HB), 0)
        for p in range(H // 2):
            b = D + p * 2 * DH
            mid = qvt[b + 16:b + 24, :]
            vt_scr[2 * p, 0:16, cols] = qvt[b:b + 16, :]
            vt_scr[2 * p, 16:24, cols] = jnp.where(sub < 4, mid, 1.0)
            vt_scr[2 * p + 1, 0:8, cols] = jnp.where(sub < 4, 1.0, mid)
            vt_scr[2 * p + 1, 8:24, cols] = qvt[b + 24:b + 40, :]
        kt = (kf_scr[cols, :].reshape(HB // 8, 8, D) * kinv_scr[...][None]).reshape(HB, D)
        la, l8, lf = [_pack8(y) for y in _limbs(kt)]
        lane = _iota((HB // 4, LANES), 1)
        krows = pl.ds(pl.multiple_of((i * RB + t * HB) // 4, HB // 4), HB // 4)
        for h in range(H):
            off = (h * DH) % 8
            g, a = divmod(h * DH, LANES)

            def place(l, r):
                src = l[:, g * LANES:(g + 1) * LANES]
                if a + DH > LANES:
                    src = jnp.where(lane >= LANES // 2, src, l[:, (g + 1) * LANES:(g + 2) * LANES])
                shift = (32 * r + off - a) % LANES
                return pltpu.roll(src, shift, 1) if shift else src

            lo = jnp.where(lane < 32, place(la, 0), place(la, 1))
            hi = jnp.where(lane < 96, place(lf, 2), place(l8, 3))
            k8_scr[h, krows, :] = jnp.where(lane < 64, lo, hi)

    def b_attention():
        n_stage = NQB * H

        def qcols(i, part):
            return pl.ds(pl.multiple_of((i >> 5) * TQ + part * W, W), W)

        def qk_chunk(i, slot, c, mx, part):
            h = i & (H - 1)
            k = pltpu.bitcast(k8_scr[h, c * KC // 4:(c + 1) * KC // 4, :], I8)
            q = pltpu.bitcast(qw_scr[h, :, qcols(i, part)], I8)
            acc = jnp.dot(k, q, preferred_element_type=I32)
            s = pltpu.bitcast(acc.reshape(KC // 8, 8, W) + mg_scr[h, :, qcols(i, part)][None], F32)
            s_scr[slot, c * KC:(c + 1) * KC, part * W:(part + 1) * W] = s.reshape(KC, W)
            cm = jnp.max(s, axis=0)
            return cm if mx is None else jnp.maximum(mx, cm)

        def store_max(slot, mx, part):
            mx_scr[slot, :, part * W:(part + 1) * W] = jnp.broadcast_to(
                jnp.max(mx, axis=0, keepdims=True), (8, W))

        def pv_chunk(i, slot, c, o, part):
            ls = slice(part * W, (part + 1) * W)
            for sub in range(KC // PKC):
                ks = slice(c * KC + sub * PKC, c * KC + (sub + 1) * PKC)
                s = s_scr[slot, ks, ls].reshape(PKC // 8, 8, W) - mx_scr[slot, :, ls][None]
                p = jnp.exp2(s).reshape(PKC, W)
                oc = jnp.dot(vt_scr[i & (H - 1), :, ks], p, preferred_element_type=F32)
                o = oc if o is None else o + oc
            return o

        def store_o(i, odd, o, part):
            p = (i & (H - 1)) >> 1
            if odd:
                ot_scr[p, DH:2 * DH, qcols(i, part)] = o[4:VR, :] * (1.0 / o[0:1, :])
            else:
                ot_scr[p, 0:DH, qcols(i, part)] = o[0:DH, :] * (1.0 / o[DH:DH + 1, :])

        for part in range(NS):
            mx = None
            for c in range(NC):
                mx = qk_chunk(0, 0, c, mx, part)
            store_max(0, mx, part)
        mx_scr[1] = jnp.zeros((8, TQ), F32)
        s_scr[1, S - KC:S, :] = jnp.zeros((KC, TQ), F32)
        oacc_scr[...] = jnp.zeros_like(oacc_scr)

        def body(j, carry):
            o = [oacc_scr[:, p * W:(p + 1) * W] for p in range(NS)]
            for u in range(UNROLL):
                i = j * UNROLL + u
                sq = (u + 1) % 2
                iq = jnp.minimum(i + 1, n_stage - 1)
                mx = [None] * NS
                for c in range(NC):
                    for part in range(NS):
                        mx[part] = qk_chunk(iq, sq, c, mx[part], part)
                        pp = (part + NS // 2) % NS
                        if c == 0:
                            ip = jnp.maximum(i - 1, 1) if u == 0 else i - 1
                            store_o(ip, sq == 1, pv_chunk(ip, sq, NC - 1, o[pp], pp), pp)
                            o[pp] = None
                        else:
                            o[pp] = pv_chunk(i, u % 2, c - 1, o[pp], pp)
                for part in range(NS):
                    store_max(sq, mx[part], part)
            for p in range(NS):
                oacc_scr[:, p * W:(p + 1) * W] = o[p]
            return carry

        jax.lax.fori_loop(0, n_stage // UNROLL, body, 0)
        for part in range(NS):
            o = pv_chunk(n_stage - 1, 1, NC - 1, oacc_scr[:, part * W:(part + 1) * W], part)
            store_o(n_stage - 1, True, o, part)

    def b_out(i, t):
        o = ot_scr[:, :, half(i, t)].reshape(D, HB).T.astype(BF16)
        return jnp.dot(o, bwo[...], preferred_element_type=F32)

    def residual_ln(i, t, out):
        x = x_scr[half(i, t), :] + out
        x_scr[half(i, t), :] = x
        return _layernorm(x).astype(BF16)

    cp_awk.start()
    x_copy(0).start()
    cp_awq.start()
    a_zero()
    cp_awk.wait()
    awkt[...] = awqkv[:, D:2 * D].T
    cp_awq.wait()
    for i in range(1, NRB):
        x_copy(i).start()
    cp_awv.start()
    cp_awo.start()
    cp_bwqkv.start()
    cp_bwo.start()

    def p1a(i, c):
        x_copy(i).wait()
        xns = []
        for t in range(RB // HB):
            x = xio[half(i, t), :].astype(F32)
            x_scr[half(i, t), :] = x
            xns.append(_layernorm(x).astype(BF16))
        a_proj(i, xns)
        return c

    jax.lax.fori_loop(0, NRB, p1a, 0)

    cp_awv.wait()
    cp_awo.wait()
    cp_bwqkv.wait()
    cp_bwo.wait()
    bwqvt[0:D, :] = bwqkv[:, 0:D].T
    bwqvt[D:2 * D, :] = bwqkv[:, 2 * D:3 * D].T

    def p2a(i, c):
        xns = [residual_ln(i, t, a_out(i, t)) for t in range(RB // HB)]
        a_norm(jnp.minimum(i + 1, NRB - 1))
        for t in range(RB // HB):
            xn_scr[half(i, t), :] = xns[t]
            b_proj_k(i, t, xns[t])
        return c

    def p2b(i, c):
        for t in range(RB // HB):
            b_proj_qv(i, t)
        return c

    def p1b(i, c):
        xns = [residual_ln(i, t, b_out(i, t)) for t in range(RB // HB)]
        a_proj(i, xns)
        return c

    def p3(i, c):
        for t in range(RB // HB):
            x = x_scr[half(i, t), :] + b_out(i, t)
            xio[half(i, t), :] = x.astype(BF16)
        o_copy(i).start()
        return c

    def layer_pair(l, c):
        a_mid()
        jax.lax.fori_loop(0, NRB, p2a, 0)
        b_mid()
        jax.lax.fori_loop(0, NRB, p2b, 0)
        b_attention()

        @pl.when(l == 0)
        def _():
            a_zero()
            jax.lax.fori_loop(0, NRB, p1b, 0)

        @pl.when(l == 1)
        def _():
            jax.lax.fori_loop(0, NRB, p3, 0)

        return c

    jax.lax.fori_loop(0, 2, layer_pair, 0)
    for i in range(NRB):
        o_copy(i).wait()


@jax.jit
def pallas_interleave_layers__linear_attn_block__mha_block__prompt_kernel(
    A_x: jax.Array,
    A_wqkv: jax.Array,
    A_wo: jax.Array,
    B_x: jax.Array,
    B_wqkv: jax.Array,
    B_wo: jax.Array,
):
    del B_x
    x = A_x.reshape(S, D)

    scratch = [
        pltpu.VMEM((S, D), BF16),
        pltpu.VMEM((D, 3 * D), BF16),
        pltpu.VMEM((D, D), BF16),
        pltpu.VMEM((D, 3 * D), BF16),
        pltpu.VMEM((D, D), BF16),
        pltpu.VMEM((D, D), BF16),
        pltpu.VMEM((2 * D, D), BF16),
        pltpu.VMEM((S, D), F32),
        pltpu.VMEM((S, D), BF16),
        pltpu.VMEM((S, D), BF16),
        pltpu.VMEM((D, D), F32),
        pltpu.VMEM((D, LANES), F32),
        pltpu.VMEM((D, D), BF16),
        pltpu.VMEM((D, LANES), BF16),
        pltpu.VMEM((S, D), BF16),
        pltpu.VMEM((S, D), F32),
        pltpu.VMEM((8, D), F32),
        pltpu.VMEM((8, D), F32),
        pltpu.VMEM((D, LANES), F32),
        pltpu.VMEM((H, LANES // 4, S), U32),
        pltpu.VMEM((H, 8, S), I32),
        pltpu.VMEM((H, S // 4, LANES), U32),
        pltpu.VMEM((H, VR, S), F32),
        pltpu.VMEM((2, S, TQ), F32),
        pltpu.VMEM((2, 8, TQ), F32),
        pltpu.VMEM((VR, TQ), F32),
        pltpu.VMEM((H // 2, 2 * DH, S), F32),
        pltpu.SemaphoreType.DMA((NRB,)),
        pltpu.SemaphoreType.DMA((6,)),
        pltpu.SemaphoreType.DMA((NRB,)),
    ]
    any_spec = pl.BlockSpec(memory_space=pl.ANY)
    out = pl.pallas_call(
        _kernel,
        out_shape=jax.ShapeDtypeStruct((S, D), A_x.dtype),
        in_specs=[any_spec] * 5,
        out_specs=any_spec,
        scratch_shapes=scratch,
        compiler_params=pltpu.CompilerParams(vmem_limit_bytes=100 * 1024 * 1024),
    )(x, A_wqkv, A_wo, B_wqkv, B_wo)
    return out.reshape(1, S, D)
```

```python
import math

import jax
import jax.numpy as jnp
import jax.experimental.pallas as pl
import jax.experimental.pallas.tpu as pltpu

S = 2048
D = 640
H = 32
DH = 20
LANES = 128
NDT = D // LANES
RB = 512
HB = 128
OB = 256
KG = 32
NRB = S // RB
TQ = 512
NQB = S // TQ
KC = 512
PKC = 128
NS = 2
W = TQ // NS
NC = S // KC
VR = 24
UNROLL = 16
EPS = 1e-5
assert RB == TQ and RB == 2 * OB and KC == 4 * LANES

NT = (((1,), (1,)), ((), ()))

BF16 = jnp.bfloat16
F32 = jnp.float32
U32 = jnp.uint32
I32 = jnp.int32
I8 = jnp.int8

RND = 12582912.0


def _phi(t):
    return jnp.where(t > 0, t + 1.0, jnp.exp(t)) + 1e-6


def _layernorm(x):
    m = jnp.mean(x, axis=-1, keepdims=True)
    xc = x - m
    v = jnp.mean(xc * xc, axis=-1, keepdims=True)
    return xc * jax.lax.rsqrt(v + EPS)


def _kv_windows():
    wins = []
    for j in range(NDT):
        h0 = (j * LANES) // DH
        h1 = (j * LANES + LANES - 1) // DH
        lo = (h0 * DH) // 16 * 16
        hi = -(-((h1 + 1) * DH) // 16) * 16
        wins.append((lo, hi))
    return wins


WINS = _kv_windows()


def _iota(shape, dim):
    return jax.lax.broadcasted_iota(jnp.int32, shape, dim)


def _pack8(v):
    return pltpu.bitcast(v.astype(I8), U32)


def _limbs(t16):
    m = pltpu.bitcast(t16 + (RND + 8.0), I32)
    return m >> 4, (m + 56) >> 7, (m & 15) - 8


def _kernel(x_hbm, awqkv_hbm, awo_hbm, bwqkv_hbm, bwo_hbm, o_hbm,
            xio, awqkv, awo, bwqkv, bwo, awkt, bwqvt,
            x_scr, pq_scr, y_scr, g_scr, z_scr, mw_scr, zt_scr,
            xn_scr, kf_scr, ksc_scr,
            qw_scr, mg_scr, k8_scr, vt_scr, s_scr, ot_scr, mx_scr, oacc_scr,
            pre_scr, kmax_scr, kinv_scr,
            xsem, wsem, osem):

    def piece(i, t):
        return pl.ds(pl.multiple_of(i * RB + t * HB, HB), HB)

    def piece2(i, t):
        return pl.ds(pl.multiple_of((i * RB + t * HB) // 2, HB // 2), HB // 2)

    def x_copy(i, first):
        if first:
            rows, sem = piece(i, 0), xsem.at[i]
        else:
            rows, sem = pl.ds(pl.multiple_of(i * RB + HB, HB), RB - HB), xsem.at[NRB + i]
        return pltpu.make_async_copy(x_hbm.at[rows, :], xio.at[rows, :], sem)

    def o_copy(n):
        rows = pl.ds(pl.multiple_of(n * OB, OB), OB)
        return pltpu.make_async_copy(xio.at[rows, :], o_hbm.at[rows, :], osem.at[n])

    cp_awk = pltpu.make_async_copy(awqkv_hbm.at[:, D:2 * D], awqkv.at[:, D:2 * D], wsem.at[0])
    cp_awq = pltpu.make_async_copy(awqkv_hbm.at[:, 0:D], awqkv.at[:, 0:D], wsem.at[1])
    cp_awv = pltpu.make_async_copy(awqkv_hbm.at[:, 2 * D:3 * D], awqkv.at[:, 2 * D:3 * D], wsem.at[2])
    cp_awo = pltpu.make_async_copy(awo_hbm, awo, wsem.at[3])
    cp_bwqkv = pltpu.make_async_copy(bwqkv_hbm, bwqkv, wsem.at[4])
    cp_bwo = pltpu.make_async_copy(bwo_hbm, bwo, wsem.at[5])

    def a_proj(i, xns):
        pkts = []
        for xn in xns:
            kt = jax.lax.dot_general(pltpu.bitcast(awkt[...], BF16), xn, NT,
                                     preferred_element_type=F32)
            pkts.append(_phi(kt))
        for t, xn in enumerate(xns):
            q = jnp.dot(xn, awqkv[:, 0:D], preferred_element_type=F32)
            pq_scr[piece2(i, t), :] = pltpu.bitcast(_phi(q).astype(BF16), U32)
        pkt = jnp.concatenate(pkts, axis=1)
        zacc = pkt[:, 0:LANES]
        for t in range(1, RB // LANES):
            zacc = zacc + pkt[:, t * LANES:(t + 1) * LANES]
        z_scr[...] += zacc
        g_scr[...] += jnp.dot(pkt.astype(BF16), jnp.concatenate(xns, axis=0),
                              preferred_element_type=F32)

    def a_norm(i):
        for t in range(RB // HB):
            pq = pltpu.bitcast(pq_scr[piece2(i, t), :], BF16)
            dent = jax.lax.dot_general(zt_scr[0:H, :], pq, NT, preferred_element_type=F32) + 1e-6
            rt = 1.0 / dent
            r = jnp.concatenate([rt] * (LANES // H), axis=0).T
            r_exp = jnp.concatenate(
                [jnp.take_along_axis(r, (_iota((HB, LANES), 1) + j * LANES) // DH, axis=1)
                 for j in range(NDT)], axis=1)
            y_scr[piece2(i, t), :] = pltpu.bitcast((pq.astype(F32) * r_exp).astype(BF16), U32)

    def a_mid():
        z = jnp.sum(z_scr[...].T, axis=0, keepdims=True)
        r0 = _iota((H, D), 0) * DH
        col = _iota((H, D), 1)
        zt_scr[0:H, :] = jnp.where((col >= r0) & (col < r0 + DH), z, 0.0).astype(BF16)
        a_norm(0)
        g = g_scr[...].astype(BF16)
        kvs = []
        for j, (lo, hi) in enumerate(WINS):
            n = hi - lo
            kvj = jnp.dot(g[lo:hi, :], awqkv[:, 2 * D + j * LANES:2 * D + (j + 1) * LANES],
                          preferred_element_type=F32)
            c0 = (_iota((1, LANES), 1) + j * LANES) // DH * DH - lo
            row = _iota((n, LANES), 0)
            kvs.append(jnp.where((row >= c0) & (row < c0 + DH), kvj, 0.0).astype(BF16))
        parts = [jnp.dot(kvs[j], awo[j * LANES:(j + 1) * LANES, :], preferred_element_type=F32)
                 for j in range(NDT)]
        for j, (lo, hi) in enumerate(WINS):
            s0 = lo if j == 0 else WINS[j - 1][1]
            s1 = hi if j == NDT - 1 else WINS[j + 1][0]
            mw_scr[s0 // 2:s1 // 2, :] = pltpu.bitcast(parts[j][s0 - lo:s1 - lo, :].astype(BF16), U32)
            if j < NDT - 1:
                mw_scr[s1 // 2:hi // 2, :] = pltpu.bitcast(
                    (parts[j][s1 - lo:hi - lo, :] + parts[j + 1][0:hi - s1, :]).astype(BF16), U32)
        kmax_scr[...] = jnp.zeros_like(kmax_scr)
        g_scr[...] = jnp.zeros_like(g_scr)
        z_scr[...] = jnp.zeros_like(z_scr)

    def a_out(i, t):
        return jnp.dot(pltpu.bitcast(y_scr[piece2(i, t), :], BF16), pltpu.bitcast(mw_scr[...], BF16),
                       preferred_element_type=F32)

    qscale = (DH ** -0.5) * math.log2(math.e)

    def b_proj_k(i, t, xn):
        k = jnp.dot(xn, bwqkv[:, D:2 * D], preferred_element_type=F32)
        kf_scr[piece(i, t), :] = k
        kmax_scr[...] = jnp.maximum(kmax_scr[...],
                                    jnp.max(jnp.abs(k).reshape(HB // 8, 8, D), axis=0))

    def b_scales():
        kmax = jnp.max(kmax_scr[...], axis=0, keepdims=True)
        kmax = jnp.maximum(kmax, 1e-30)
        kinv_scr[...] = jnp.broadcast_to((16.0 * 127.0) / kmax, (8, D))
        ksc_scr[...] = jnp.broadcast_to(kmax * (qscale / 127.0), (LANES, D)).T

    def b_proj_qv(i, t):
        cols = piece(i, t)
        lc = slice(t * HB, (t + 1) * HB)
        xn = pltpu.bitcast(xn_scr[piece2(i, t), :], BF16)
        qvt = jax.lax.dot_general(pltpu.bitcast(bwqvt[...], BF16), xn, NT,
                                  preferred_element_type=F32)
        row = _iota((VR, HB), 0)
        zero8 = jnp.zeros((8, HB), I32)
        for h in range(H):
            off = (h * DH) % 8
            w0 = h * DH - off
            q = jnp.where((row >= off) & (row < off + DH),
                          qvt[w0:w0 + VR, :] * ksc_scr[w0:w0 + VR, :], 0.0)
            qmax = jnp.max(jnp.abs(q), axis=0, keepdims=True) * (1.0 / 127.0)
            eb = jnp.clip(pltpu.bitcast(qmax, I32) >> 23, 66, 226)
            qa, q8, qf = _limbs(q * pltpu.bitcast((257 - eb) << 23, F32))
            pa = _pack8(jnp.concatenate([qa, zero8], axis=0))
            qw_scr[i * H + h, 0:8, lc] = pa
            qw_scr[i * H + h, 8:16, lc] = pa
            qw_scr[i * H + h, 16:24, lc] = _pack8(jnp.concatenate([q8, zero8], axis=0))
            qw_scr[i * H + h, 24:32, lc] = _pack8(jnp.concatenate([qf, zero8], axis=0))
            mg_scr[i * H + h, :, lc] = jnp.broadcast_to(((eb + 23) << 23) | 0x400000, (8, HB))
        sub = _iota((8, HB), 0)
        for p in range(H // 2):
            b = D + p * 2 * DH
            mid = qvt[b + 16:b + 24, :]
            vt_scr[2 * p, 0:16, cols] = qvt[b:b + 16, :]
            vt_scr[2 * p, 16:24, cols] = jnp.where(sub < 4, mid, 1.0)
            vt_scr[2 * p + 1, 0:8, cols] = jnp.where(sub < 4, 1.0, mid)
            vt_scr[2 * p + 1, 8:24, cols] = qvt[b + 24:b + 40, :]
        lane = _iota((KG // 4, LANES), 1)
        for n in range(HB // KG):
            r0 = i * RB + t * HB + n * KG
            kt = (kf_scr[pl.ds(pl.multiple_of(r0, KG), KG), :].reshape(KG // 8, 8, D)
                  * kinv_scr[...][None]).reshape(KG, D)
            ka, k8, kf = [_pack8(v) for v in _limbs(kt)]
            krows = pl.ds(pl.multiple_of(r0 // 4, KG // 4), KG // 4)
            for h in range(H):
                off = (h * DH) % 8
                g, a = divmod(h * DH, LANES)

                def place(l, r):
                    src = l[:, g * LANES:(g + 1) * LANES]
                    if a + DH > LANES:
                        src = jnp.where(lane >= LANES // 2, src,
                                        l[:, (g + 1) * LANES:(g + 2) * LANES])
                    shift = (32 * r + off - a) % LANES
                    return pltpu.roll(src, shift, 1) if shift else src

                lo = jnp.where(lane < 32, place(ka, 0), place(ka, 1))
                hi = jnp.where(lane < 96, place(kf, 2), place(k8, 3))
                k8_scr[h, krows, :] = jnp.where(lane < 64, lo, hi)

    def o_rows(i, t):
        cols = pl.ds(t * HB if isinstance(t, int) else pl.multiple_of(t * HB, HB), HB)
        return ot_scr[pl.ds(i * (H // 2), H // 2), :, cols].reshape(D, HB).T.astype(BF16)

    def b_attention():
        n_stage = NQB * H

        def qk_chunk(i, slot, c, mx, part):
            ls = slice(part * W, (part + 1) * W)
            k = pltpu.bitcast(k8_scr[i & (H - 1), c * KC // 4:(c + 1) * KC // 4, :], I8)
            q = pltpu.bitcast(qw_scr[i, :, ls], I8)
            acc = jnp.dot(k, q, preferred_element_type=I32)
            s = pltpu.bitcast(acc.reshape(KC // 8, 8, W) + mg_scr[i, :, ls][None], F32)
            s_scr[slot, c * KC:(c + 1) * KC, ls] = s.reshape(KC, W)
            cm = jnp.max(s, axis=0)
            return cm if mx is None else jnp.maximum(mx, cm)

        def store_max(slot, mx, part):
            mx_scr[slot, :, part * W:(part + 1) * W] = jnp.broadcast_to(
                jnp.max(mx, axis=0, keepdims=True), (8, W))

        def pv_chunk(i, slot, c, o, part):
            ls = slice(part * W, (part + 1) * W)
            for sub in range(KC // PKC):
                ks = slice(c * KC + sub * PKC, c * KC + (sub + 1) * PKC)
                s = s_scr[slot, ks, ls].reshape(PKC // 8, 8, W) - mx_scr[slot, :, ls][None]
                p = jnp.exp2(s).reshape(PKC, W)
                oc = jnp.dot(vt_scr[i & (H - 1), :, ks], p, preferred_element_type=F32,
                             precision=jax.lax.Precision.DEFAULT)
                o = oc if o is None else o + oc
            return o

        def store_o(i, odd, o, part):
            ls = slice(part * W, (part + 1) * W)
            if odd:
                ot_scr[i >> 1, DH:2 * DH, ls] = o[4:VR, :] * (1.0 / o[0:1, :])
            else:
                ot_scr[i >> 1, 0:DH, ls] = o[0:DH, :] * (1.0 / o[DH:DH + 1, :])

        for part in range(NS):
            mx = None
            for c in range(NC):
                mx = qk_chunk(0, 0, c, mx, part)
            store_max(0, mx, part)

        def body(j, carry):
            o = [oacc_scr[:, p * W:(p + 1) * W] for p in range(NS)]
            for u in range(UNROLL):
                i = j * UNROLL + u
                sq = (u + 1) % 2
                iq = jnp.minimum(i + 1, n_stage - 1)
                mx = [None] * NS
                for c in range(NC):
                    for part in range(NS):
                        mx[part] = qk_chunk(iq, sq, c, mx[part], part)
                        pp = (part + NS // 2) % NS
                        if c == 0:
                            ip = jnp.maximum(i - 1, 1) if u == 0 else i - 1
                            store_o(ip, sq == 1, pv_chunk(ip, sq, NC - 1, o[pp], pp), pp)
                            o[pp] = None
                        else:
                            o[pp] = pv_chunk(i, u % 2, c - 1, o[pp], pp)
                for part in range(NS):
                    store_max(sq, mx[part], part)
            for p in range(NS):
                oacc_scr[:, p * W:(p + 1) * W] = o[p]
            return carry

        jax.lax.fori_loop(0, n_stage // UNROLL, body, 0)
        for part in range(NS):
            o = pv_chunk(n_stage - 1, 1, NC - 1, oacc_scr[:, part * W:(part + 1) * W], part)
            store_o(n_stage - 1, True, o, part)
        pre_scr[...] = pltpu.bitcast(o_rows(0, 0), U32)

    def b_out(i, t, first):
        o = pltpu.bitcast(pre_scr[...], BF16) if first else o_rows(i, t)
        return jnp.dot(o, bwo[...], preferred_element_type=F32)

    def residual_ln(i, t, out):
        x = x_scr[piece(i, t), :] + out
        x_scr[piece(i, t), :] = x
        return _layernorm(x).astype(BF16)

    def load_ln(i, t):
        x = xio[piece(i, t), :].astype(F32)
        x_scr[piece(i, t), :] = x
        return _layernorm(x).astype(BF16)

    x_copy(0, True).start()
    cp_awk.start()
    x_copy(0, False).start()
    cp_awq.start()
    x_copy(1, True).start()

    def zero_body(n, c):
        rows = pl.ds(pl.multiple_of(n * LANES, LANES), LANES)
        g_scr[rows, :] = jnp.zeros((LANES, D), F32)
        z_scr[rows, :] = jnp.zeros((LANES, LANES), F32)
        srows = pl.ds(pl.multiple_of(S - KC + jnp.minimum(n, 3) * LANES, LANES), LANES)
        s_scr[1, srows, :] = jnp.zeros((LANES, TQ), F32)
        return c

    jax.lax.fori_loop(0, NDT, zero_body, 0)
    mx_scr[1] = jnp.zeros((8, TQ), F32)
    oacc_scr[...] = jnp.zeros_like(oacc_scr)
    x_copy(0, True).wait()
    pre_scr[...] = pltpu.bitcast(load_ln(0, 0), U32)
    cp_awk.wait()
    awkt[...] = pltpu.bitcast(awqkv[:, D:2 * D].T, U32)
    cp_awq.wait()
    for i in range(1, NRB):
        x_copy(i, False).start()
        if i + 1 < NRB:
            x_copy(i + 1, True).start()
    cp_awv.start()
    cp_awo.start()
    cp_bwqkv.start()
    cp_bwo.start()

    def p1a(i, c):
        x_copy(i, False).wait()

        @pl.when(i + 1 < NRB)
        def _():
            x_copy(i + 1, True).wait()

        xns = [pltpu.bitcast(pre_scr[...], BF16)] + [load_ln(i, t) for t in range(1, RB // HB)]
        a_proj(i, xns)
        pre_scr[...] = pltpu.bitcast(load_ln(jnp.minimum(i + 1, NRB - 1), 0), U32)
        return c

    jax.lax.fori_loop(0, NRB, p1a, 0)

    cp_awv.wait()
    cp_awo.wait()
    cp_bwqkv.wait()
    cp_bwo.wait()

    def p2a(i, c):
        xns = [residual_ln(i, t, a_out(i, t)) for t in range(RB // HB)]
        a_norm(jnp.minimum(i + 1, NRB - 1))
        for t in range(RB // HB):
            xn_scr[piece2(i, t), :] = pltpu.bitcast(xns[t], U32)
            b_proj_k(i, t, xns[t])
        per = -(-2 * NDT // NRB)
        for n in range(per):
            tile = jnp.minimum(i * per + n, 2 * NDT - 1)
            c0 = pl.multiple_of(jnp.where(tile < NDT, tile, tile + NDT) * LANES, LANES)
            bwqvt[pl.ds(pl.multiple_of(tile * (LANES // 2), LANES // 2), LANES // 2), :] = pltpu.bitcast(
                bwqkv[:, pl.ds(c0, LANES)].T, U32)
        return c

    def p2b(i, c):
        b_scales()
        for t in range(RB // HB):
            b_proj_qv(i, t)
        return c

    def p1b(i, c):
        xns = [residual_ln(i, t, b_out(i, t, t == 0)) for t in range(RB // HB)]
        a_proj(i, xns)
        pre_scr[...] = pltpu.bitcast(o_rows(jnp.minimum(i + 1, NRB - 1), 0), U32)
        return c

    def p3(n, c):
        i = n >> 1
        for e in range(OB // HB):
            t = (n & 1) * (OB // HB) + e
            x = x_scr[piece(i, t), :] + b_out(i, t, e == 0)
            xio[piece(i, t), :] = x.astype(BF16)
        nn = jnp.minimum(n + 1, S // OB - 1)
        pre_scr[...] = pltpu.bitcast(o_rows(nn >> 1, (nn & 1) * (OB // HB)), U32)
        o_copy(n).start()
        return c

    def layer_pair(l, c):
        a_mid()
        jax.lax.fori_loop(0, NRB, p2a, 0)
        jax.lax.fori_loop(0, NRB, p2b, 0)
        b_attention()

        @pl.when(l == 0)
        def _():
            jax.lax.fori_loop(0, NRB, p1b, 0)

        @pl.when(l == 1)
        def _():
            jax.lax.fori_loop(0, S // OB, p3, 0)

        return c

    jax.lax.fori_loop(0, 2, layer_pair, 0)
    for n in range(S // OB):
        o_copy(n).wait()


@jax.jit
def pallas_interleave_layers__linear_attn_block__mha_block__prompt_kernel(
    A_x: jax.Array,
    A_wqkv: jax.Array,
    A_wo: jax.Array,
    B_x: jax.Array,
    B_wqkv: jax.Array,
    B_wo: jax.Array,
):
    del B_x
    x = A_x.reshape(S, D)

    scratch = [
        pltpu.VMEM((S, D), BF16),
        pltpu.VMEM((D, 3 * D), BF16),
        pltpu.VMEM((D, D), BF16),
        pltpu.VMEM((D, 3 * D), BF16),
        pltpu.VMEM((D, D), BF16),
        pltpu.VMEM((D // 2, D), U32),
        pltpu.VMEM((D, D), U32),
        pltpu.VMEM((S, D), F32),
        pltpu.VMEM((S // 2, D), U32),
        pltpu.VMEM((S // 2, D), U32),
        pltpu.VMEM((D, D), F32),
        pltpu.VMEM((D, LANES), F32),
        pltpu.VMEM((D // 2, D), U32),
        pltpu.VMEM((LANES, D), BF16),
        pltpu.VMEM((S // 2, D), U32),
        pltpu.VMEM((S, D), F32),
        pltpu.VMEM((D, LANES), F32),
        pltpu.VMEM((NQB * H, LANES // 4, TQ), U32),
        pltpu.VMEM((NQB * H, 8, TQ), I32),
        pltpu.VMEM((H, S // 4, LANES), U32),
        pltpu.VMEM((H, VR, S), F32),
        pltpu.VMEM((2, S, TQ), F32),
        pltpu.VMEM((NQB * H // 2, 2 * DH, TQ), F32),
        pltpu.VMEM((2, 8, TQ), F32),
        pltpu.VMEM((VR, TQ), F32),
        pltpu.VMEM((HB // 2, D), U32),
        pltpu.VMEM((8, D), F32),
        pltpu.VMEM((8, D), F32),
        pltpu.SemaphoreType.DMA((2 * NRB,)),
        pltpu.SemaphoreType.DMA((6,)),
        pltpu.SemaphoreType.DMA((S // OB,)),
    ]
    any_spec = pl.BlockSpec(memory_space=pl.ANY)
    out = pl.pallas_call(
        _kernel,
        out_shape=jax.ShapeDtypeStruct((S, D), A_x.dtype),
        in_specs=[any_spec] * 5,
        out_specs=any_spec,
        scratch_shapes=scratch,
        compiler_params=pltpu.CompilerParams(vmem_limit_bytes=100 * 1024 * 1024),
    )(x, A_wqkv, A_wo, B_wqkv, B_wo)
    return out.reshape(1, S, D)
```

```python
import math

import jax
import jax.numpy as jnp
import jax.experimental.pallas as pl
import jax.experimental.pallas.tpu as pltpu

S = 2048
D = 640
H = 32
DH = 20
LANES = 128
NDT = D // LANES
RB = 512
HB = 128
OB = 256
KG = 32
NRB = S // RB
TQ = 512
NQB = S // TQ
KC = 512
PKC = 128
LEAD = (1, 3, 4, 0)
NS = len(LEAD)
W = TQ // NS
NC = S // KC
VR = 24
UNROLL = 16
NPRE = 3
KVFIRST = 2
EPS = 1e-5
assert RB == TQ and RB == 2 * OB and KC == 4 * LANES

NT = (((1,), (1,)), ((), ()))

BF16 = jnp.bfloat16
F32 = jnp.float32
U32 = jnp.uint32
I32 = jnp.int32
I8 = jnp.int8

RND = 12582912.0


def _phi(t):
    return jnp.where(t > 0, t + 1.0, jnp.exp(t)) + 1e-6


def _layernorm(x):
    m = jnp.mean(x, axis=-1, keepdims=True)
    xc = x - m
    v = jnp.mean(xc * xc, axis=-1, keepdims=True)
    return xc * jax.lax.rsqrt(v + EPS)


def _kv_windows():
    wins = []
    for j in range(NDT):
        h0 = (j * LANES) // DH
        h1 = (j * LANES + LANES - 1) // DH
        lo = (h0 * DH) // 16 * 16
        hi = -(-((h1 + 1) * DH) // 16) * 16
        wins.append((lo, hi))
    return wins


WINS = _kv_windows()


def _iota(shape, dim):
    return jax.lax.broadcasted_iota(jnp.int32, shape, dim)


def _pack8(v):
    return pltpu.bitcast(v.astype(I8), U32)


def _limbs(t16):
    m = pltpu.bitcast(t16 + (RND + 8.0), I32)
    return m >> 4, (m + 56) >> 7, (m & 15) - 8


def _kernel(x_hbm, awqkv_hbm, awo_hbm, bwqkv_hbm, bwo_hbm, o_hbm,
            xio, awqkv, awo, bwqkv, bwo, awkt, bwqvt,
            x_scr, pq_scr, y_scr, g_scr, z_scr, mw_scr, zt_scr,
            xn_scr, kf_scr, ksc_scr,
            qw_scr, mg_scr, k8_scr, vt_scr, s_scr, ot_scr, mx_scr, mxc_scr, oacc_scr,
            pre_scr, kmax_scr, kinv_scr,
            xsem, wsem, osem):

    def piece(i, t):
        return pl.ds(pl.multiple_of(i * RB + t * HB, HB), HB)

    def piece2(i, t):
        return pl.ds(pl.multiple_of((i * RB + t * HB) // 2, HB // 2), HB // 2)

    def x_copy(i, first):
        if first:
            rows, sem = piece(i, 0), xsem.at[i]
        else:
            rows, sem = pl.ds(pl.multiple_of(i * RB + HB, HB), RB - HB), xsem.at[NRB + i]
        return pltpu.make_async_copy(x_hbm.at[rows, :], xio.at[rows, :], sem)

    def o_copy(n):
        rows = pl.ds(pl.multiple_of(n * OB, OB), OB)
        return pltpu.make_async_copy(xio.at[rows, :], o_hbm.at[rows, :], osem.at[n])

    cp_awk = pltpu.make_async_copy(awqkv_hbm.at[:, D:2 * D], awqkv.at[:, D:2 * D], wsem.at[0])
    cp_awq = pltpu.make_async_copy(awqkv_hbm.at[:, 0:D], awqkv.at[:, 0:D], wsem.at[1])
    cp_awv = pltpu.make_async_copy(awqkv_hbm.at[:, 2 * D:3 * D], awqkv.at[:, 2 * D:3 * D], wsem.at[2])
    cp_awo = pltpu.make_async_copy(awo_hbm, awo, wsem.at[3])
    cp_bwqkv = pltpu.make_async_copy(bwqkv_hbm, bwqkv, wsem.at[4])
    cp_bwo = pltpu.make_async_copy(bwo_hbm, bwo, wsem.at[5])

    def a_proj(i, xns):
        pkts = []
        for xn in xns:
            kt = jax.lax.dot_general(pltpu.bitcast(awkt[...], BF16), xn, NT,
                                     preferred_element_type=F32)
            pkts.append(_phi(kt))
        for t, xn in enumerate(xns):
            q = jnp.dot(xn, awqkv[:, 0:D], preferred_element_type=F32)
            pq_scr[piece2(i, t), :] = pltpu.bitcast(_phi(q).astype(BF16), U32)
        pkt = jnp.concatenate(pkts, axis=1)
        zacc = pkt[:, 0:LANES]
        for t in range(1, RB // LANES):
            zacc = zacc + pkt[:, t * LANES:(t + 1) * LANES]
        z_scr[...] += zacc
        g_scr[...] += jnp.dot(pkt.astype(BF16), jnp.concatenate(xns, axis=0),
                              preferred_element_type=F32)

    def a_y(i, t):
        pq = pltpu.bitcast(pq_scr[piece2(i, t), :], BF16)
        dent = jax.lax.dot_general(zt_scr[0:H, :], pq, NT, preferred_element_type=F32) + 1e-6
        rt = 1.0 / dent
        r = jnp.concatenate([rt] * (LANES // H), axis=0).T
        r_exp = jnp.concatenate(
            [jnp.take_along_axis(r, (_iota((HB, LANES), 1) + j * LANES) // DH, axis=1)
             for j in range(NDT)], axis=1)
        return (pq.astype(F32) * r_exp).astype(BF16)

    def a_norm(i):
        for t in range(NPRE):
            y_scr[t] = pltpu.bitcast(a_y(i, t), U32)

    def a_mid():
        kvs = []
        for j, (lo, hi) in enumerate(WINS):
            if j == KVFIRST:
                z = jnp.sum(z_scr[...].T, axis=0, keepdims=True)
                r0 = _iota((H, D), 0) * DH
                col = _iota((H, D), 1)
                zt_scr[0:H, :] = jnp.where((col >= r0) & (col < r0 + DH), z, 0.0).astype(BF16)
                a_norm(0)
            n = hi - lo
            kvj = jnp.dot(g_scr[lo:hi, :].astype(BF16),
                          awqkv[:, 2 * D + j * LANES:2 * D + (j + 1) * LANES],
                          preferred_element_type=F32)
            c0 = (_iota((1, LANES), 1) + j * LANES) // DH * DH - lo
            row = _iota((n, LANES), 0)
            kvs.append(jnp.where((row >= c0) & (row < c0 + DH), kvj, 0.0).astype(BF16))
        parts = [jnp.dot(kvs[j], awo[j * LANES:(j + 1) * LANES, :], preferred_element_type=F32)
                 for j in range(NDT)]
        for j, (lo, hi) in enumerate(WINS):
            s0 = lo if j == 0 else WINS[j - 1][1]
            s1 = hi if j == NDT - 1 else WINS[j + 1][0]
            mw_scr[s0 // 2:s1 // 2, :] = pltpu.bitcast(parts[j][s0 - lo:s1 - lo, :].astype(BF16), U32)
            if j < NDT - 1:
                mw_scr[s1 // 2:hi // 2, :] = pltpu.bitcast(
                    (parts[j][s1 - lo:hi - lo, :] + parts[j + 1][0:hi - s1, :]).astype(BF16), U32)
        kmax_scr[...] = jnp.zeros_like(kmax_scr)
        g_scr[...] = jnp.zeros_like(g_scr)
        z_scr[...] = jnp.zeros_like(z_scr)

    def a_out(y):
        return jnp.dot(y, pltpu.bitcast(mw_scr[...], BF16), preferred_element_type=F32)

    qscale = (DH ** -0.5) * math.log2(math.e)

    def b_proj_k(i, t, xn):
        k = jnp.dot(xn, bwqkv[:, D:2 * D], preferred_element_type=F32)
        kf_scr[piece(i, t), :] = k
        kmax_scr[...] = jnp.maximum(kmax_scr[...],
                                    jnp.max(jnp.abs(k).reshape(HB // 8, 8, D), axis=0))

    def b_scales():
        kmax = jnp.max(kmax_scr[...], axis=0, keepdims=True)
        kmax = jnp.maximum(kmax, 1e-30)
        kinv_scr[...] = jnp.broadcast_to((16.0 * 127.0) / kmax, (8, D))
        ksc_scr[...] = jnp.broadcast_to(kmax * (qscale / 127.0), (LANES, D)).T

    def b_proj_qv(i, t):
        cols = piece(i, t)
        lc = slice(t * HB, (t + 1) * HB)
        xn = pltpu.bitcast(xn_scr[piece2(i, t), :], BF16)
        qvt = jax.lax.dot_general(pltpu.bitcast(bwqvt[...], BF16), xn, NT,
                                  preferred_element_type=F32)
        row = _iota((VR, HB), 0)
        zero8 = jnp.zeros((8, HB), I32)
        for h in range(H):
            off = (h * DH) % 8
            w0 = h * DH - off
            q = jnp.where((row >= off) & (row < off + DH),
                          qvt[w0:w0 + VR, :] * ksc_scr[w0:w0 + VR, :], 0.0)
            qmax = jnp.max(jnp.abs(q), axis=0, keepdims=True) * (1.0 / 127.0)
            eb = jnp.clip(pltpu.bitcast(qmax, I32) >> 23, 66, 226)
            qa, q8, qf = _limbs(q * pltpu.bitcast((257 - eb) << 23, F32))
            pa = _pack8(jnp.concatenate([qa, zero8], axis=0))
            qw_scr[i * H + h, 0:8, lc] = pa
            qw_scr[i * H + h, 8:16, lc] = pa
            qw_scr[i * H + h, 16:24, lc] = _pack8(jnp.concatenate([q8, zero8], axis=0))
            qw_scr[i * H + h, 24:32, lc] = _pack8(jnp.concatenate([qf, zero8], axis=0))
            mg_scr[i * H + h, :, lc] = jnp.broadcast_to(((eb + 23) << 23) | 0x400000, (8, HB))
        sub = _iota((8, HB), 0)
        for p in range(H // 2):
            b = D + p * 2 * DH
            mid = qvt[b + 16:b + 24, :]
            vt_scr[2 * p, 0:16, cols] = qvt[b:b + 16, :]
            vt_scr[2 * p, 16:24, cols] = jnp.where(sub < 4, mid, 1.0)
            vt_scr[2 * p + 1, 0:8, cols] = jnp.where(sub < 4, 1.0, mid)
            vt_scr[2 * p + 1, 8:24, cols] = qvt[b + 24:b + 40, :]
        lane = _iota((KG // 4, LANES), 1)
        for n in range(HB // KG):
            r0 = i * RB + t * HB + n * KG
            kt = (kf_scr[pl.ds(pl.multiple_of(r0, KG), KG), :].reshape(KG // 8, 8, D)
                  * kinv_scr[...][None]).reshape(KG, D)
            ka, k8, kf = [_pack8(v) for v in _limbs(kt)]
            krows = pl.ds(pl.multiple_of(r0 // 4, KG // 4), KG // 4)
            for h in range(H):
                off = (h * DH) % 8
                g, a = divmod(h * DH, LANES)

                def place(l, r):
                    src = l[:, g * LANES:(g + 1) * LANES]
                    if a + DH > LANES:
                        src = jnp.where(lane >= LANES // 2, src,
                                        l[:, (g + 1) * LANES:(g + 2) * LANES])
                    shift = (32 * r + off - a) % LANES
                    return pltpu.roll(src, shift, 1) if shift else src

                lo = jnp.where(lane < 32, place(ka, 0), place(ka, 1))
                hi = jnp.where(lane < 96, place(kf, 2), place(k8, 3))
                k8_scr[h, krows, :] = jnp.where(lane < 64, lo, hi)

    def o_rows(i, t):
        cols = pl.ds(t * HB if isinstance(t, int) else pl.multiple_of(t * HB, HB), HB)
        return ot_scr[pl.ds(i * (H // 2), H // 2), :, cols].reshape(D, HB).T.astype(BF16)

    def b_attention():
        n_stage = NQB * H
        upc = KC // PKC
        ups = S // PKC
        ahead = [(upc - r) % upc for r in LEAD]

        def qk(i, slot, k0, k1, mx, p):
            ls = slice(p * W, (p + 1) * W)
            n = (k1 - k0) * PKC
            k = pltpu.bitcast(k8_scr[i & (H - 1), k0 * PKC // 4:k1 * PKC // 4, :], I8)
            q = pltpu.bitcast(qw_scr[i, :, ls], I8)
            acc = jnp.dot(k, q, preferred_element_type=I32)
            s = pltpu.bitcast(acc.reshape(n // 8, 8, W) + mg_scr[i, :, ls][None], F32)
            s_scr[slot, k0 * PKC:k1 * PKC, ls] = s.reshape(n, W)
            cm = jnp.max(s, axis=0)
            mx = cm if mx is None else jnp.maximum(mx, cm)
            if k1 == ups:
                mx_scr[slot, :, ls] = jnp.broadcast_to(jnp.max(mx, axis=0, keepdims=True), (8, W))
            return mx

        def pv(i, slot, c, o, p):
            ls = slice(p * W, (p + 1) * W)
            for sub in range(upc):
                ks = slice(c * KC + sub * PKC, c * KC + (sub + 1) * PKC)
                s = s_scr[slot, ks, ls].reshape(PKC // 8, 8, W) - mx_scr[slot, :, ls][None]
                pt = jnp.exp2(s).reshape(PKC, W)
                oc = jnp.dot(vt_scr[i & (H - 1), :, ks], pt, preferred_element_type=F32,
                             precision=jax.lax.Precision.DEFAULT)
                o = oc if o is None else o + oc
            if c == NC - 1:
                if slot == 1:
                    ot_scr[i >> 1, DH:2 * DH, ls] = o[4:VR, :] * (1.0 / o[0:1, :])
                else:
                    ot_scr[i >> 1, 0:DH, ls] = o[0:DH, :] * (1.0 / o[DH:DH + 1, :])
            return o

        mx = [None] * NS
        for c in range(NC):
            for p in range(NS):
                mx[p] = qk(0, 0, c * upc, (c + 1) * upc, mx[p], p)
        for p in range(NS):
            if ahead[p]:
                mxc_scr[:, p * W:(p + 1) * W] = qk(1, 1, 0, ahead[p], None, p)

        ops = []
        for p in range(NS):
            t, n, end = 0, ahead[p], ups * UNROLL + ahead[p]
            for b in range(-1, NC * UNROLL):
                if b >= 0:
                    ops.append((t, p, "pv", b - 1, None))
                    t += 102
                take = LEAD[p] if b < 0 else min(upc, end - n)
                if take:
                    ops.append((t, p, "qk", n, n + take))
                    t, n = t + 64 * take, n + take
        ops.sort(key=lambda op: op[:2])

        def body(j, carry):
            o = [oacc_scr[:, p * W:(p + 1) * W] for p in range(NS)]
            mx = [mxc_scr[:, p * W:(p + 1) * W] if ahead[p] else None for p in range(NS)]
            for _, p, kind, a, b in ops:
                if kind == "qk":
                    u = a // ups + 1
                    i = j * UNROLL + u
                    if u >= UNROLL:
                        i = jnp.minimum(i, n_stage - 1)
                    mx[p] = qk(i, u % 2, a % ups, (b - 1) % ups + 1, mx[p] if a % ups else None, p)
                else:
                    u, c = divmod(a, NC)
                    i = j * UNROLL + u if u >= 0 else jnp.maximum(j * UNROLL + u, 1)
                    o[p] = pv(i, u % 2, c, o[p] if c else None, p)
            for p in range(NS):
                oacc_scr[:, p * W:(p + 1) * W] = o[p]
                if ahead[p]:
                    mxc_scr[:, p * W:(p + 1) * W] = mx[p]
            return carry

        jax.lax.fori_loop(0, n_stage // UNROLL, body, 0)
        for p in range(NS):
            pv(n_stage - 1, 1, NC - 1, oacc_scr[:, p * W:(p + 1) * W], p)
        pre_scr[...] = pltpu.bitcast(o_rows(0, 0), U32)

    def b_out(i, t, first):
        o = pltpu.bitcast(pre_scr[...], BF16) if first else o_rows(i, t)
        return jnp.dot(o, bwo[...], preferred_element_type=F32)

    def residual_ln(i, t, out):
        x = x_scr[piece(i, t), :] + out
        x_scr[piece(i, t), :] = x
        return _layernorm(x).astype(BF16)

    def load_ln(i, t):
        x = xio[piece(i, t), :].astype(F32)
        x_scr[piece(i, t), :] = x
        return _layernorm(x).astype(BF16)

    x_copy(0, True).start()
    cp_awk.start()
    x_copy(0, False).start()
    cp_awq.start()
    x_copy(1, True).start()

    def zero_body(n, c):
        rows = pl.ds(pl.multiple_of(n * LANES, LANES), LANES)
        g_scr[rows, :] = jnp.zeros((LANES, D), F32)
        z_scr[rows, :] = jnp.zeros((LANES, LANES), F32)
        srows = pl.ds(pl.multiple_of(S - KC + jnp.minimum(n, 3) * LANES, LANES), LANES)
        s_scr[1, srows, :] = jnp.zeros((LANES, TQ), F32)
        return c

    jax.lax.fori_loop(0, NDT, zero_body, 0)
    mx_scr[1] = jnp.zeros((8, TQ), F32)
    oacc_scr[...] = jnp.zeros_like(oacc_scr)
    x_copy(0, True).wait()
    pre_scr[...] = pltpu.bitcast(load_ln(0, 0), U32)
    cp_awk.wait()
    awkt[...] = pltpu.bitcast(awqkv[:, D:2 * D].T, U32)
    cp_awq.wait()
    for i in range(1, NRB):
        x_copy(i, False).start()
        if i + 1 < NRB:
            x_copy(i + 1, True).start()
    cp_awv.start()
    cp_awo.start()
    cp_bwqkv.start()
    cp_bwo.start()

    def p1a(i, c):
        x_copy(i, False).wait()

        @pl.when(i + 1 < NRB)
        def _():
            x_copy(i + 1, True).wait()

        xns = [pltpu.bitcast(pre_scr[...], BF16)] + [load_ln(i, t) for t in range(1, RB // HB)]
        a_proj(i, xns)
        pre_scr[...] = pltpu.bitcast(load_ln(jnp.minimum(i + 1, NRB - 1), 0), U32)
        return c

    jax.lax.fori_loop(0, NRB, p1a, 0)

    cp_awv.wait()
    cp_awo.wait()
    cp_bwqkv.wait()
    cp_bwo.wait()

    def p2a(i, c):
        ys = [pltpu.bitcast(y_scr[t], BF16) if t < NPRE else a_y(i, t)
              for t in range(RB // HB)]
        xns = [residual_ln(i, t, a_out(ys[t])) for t in range(RB // HB)]
        a_norm(jnp.minimum(i + 1, NRB - 1))
        for t in range(RB // HB):
            xn_scr[piece2(i, t), :] = pltpu.bitcast(xns[t], U32)
            b_proj_k(i, t, xns[t])
        per = -(-2 * NDT // NRB)
        for n in range(per):
            tile = jnp.minimum(i * per + n, 2 * NDT - 1)
            c0 = pl.multiple_of(jnp.where(tile < NDT, tile, tile + NDT) * LANES, LANES)
            bwqvt[pl.ds(pl.multiple_of(tile * (LANES // 2), LANES // 2), LANES // 2), :] = pltpu.bitcast(
                bwqkv[:, pl.ds(c0, LANES)].T, U32)
        return c

    def p2b(i, c):
        b_scales()
        for t in range(RB // HB):
            b_proj_qv(i, t)
        return c

    def p1b(i, c):
        xns = [residual_ln(i, t, b_out(i, t, t == 0)) for t in range(RB // HB)]
        a_proj(i, xns)
        pre_scr[...] = pltpu.bitcast(o_rows(jnp.minimum(i + 1, NRB - 1), 0), U32)
        return c

    def p3(n, c):
        i = n >> 1
        for e in range(OB // HB):
            t = (n & 1) * (OB // HB) + e
            x = x_scr[piece(i, t), :] + b_out(i, t, e == 0)
            xio[piece(i, t), :] = x.astype(BF16)
        nn = jnp.minimum(n + 1, S // OB - 1)
        pre_scr[...] = pltpu.bitcast(o_rows(nn >> 1, (nn & 1) * (OB // HB)), U32)
        o_copy(n).start()
        return c

    def layer_pair(l, c):
        a_mid()
        jax.lax.fori_loop(0, NRB, p2a, 0)
        jax.lax.fori_loop(0, NRB, p2b, 0)
        b_attention()

        @pl.when(l == 0)
        def _():
            jax.lax.fori_loop(0, NRB, p1b, 0)

        @pl.when(l == 1)
        def _():
            jax.lax.fori_loop(0, S // OB, p3, 0)

        return c

    jax.lax.fori_loop(0, 2, layer_pair, 0)
    for n in range(S // OB):
        o_copy(n).wait()


@jax.jit
def pallas_interleave_layers__linear_attn_block__mha_block__prompt_kernel(
    A_x: jax.Array,
    A_wqkv: jax.Array,
    A_wo: jax.Array,
    B_x: jax.Array,
    B_wqkv: jax.Array,
    B_wo: jax.Array,
):
    del B_x
    x = A_x.reshape(S, D)

    scratch = [
        pltpu.VMEM((S, D), BF16),
        pltpu.VMEM((D, 3 * D), BF16),
        pltpu.VMEM((D, D), BF16),
        pltpu.VMEM((D, 3 * D), BF16),
        pltpu.VMEM((D, D), BF16),
        pltpu.VMEM((D // 2, D), U32),
        pltpu.VMEM((D, D), U32),
        pltpu.VMEM((S, D), F32),
        pltpu.VMEM((S // 2, D), U32),
        pltpu.VMEM((NPRE, HB // 2, D), U32),
        pltpu.VMEM((D, D), F32),
        pltpu.VMEM((D, LANES), F32),
        pltpu.VMEM((D // 2, D), U32),
        pltpu.VMEM((LANES, D), BF16),
        pltpu.VMEM((S // 2, D), U32),
        pltpu.VMEM((S, D), F32),
        pltpu.VMEM((D, LANES), F32),
        pltpu.VMEM((NQB * H, LANES // 4, TQ), U32),
        pltpu.VMEM((NQB * H, 8, TQ), I32),
        pltpu.VMEM((H, S // 4, LANES), U32),
        pltpu.VMEM((H, VR, S), F32),
        pltpu.VMEM((2, S, TQ), F32),
        pltpu.VMEM((NQB * H // 2, 2 * DH, TQ), F32),
        pltpu.VMEM((2, 8, TQ), F32),
        pltpu.VMEM((8, TQ), F32),
        pltpu.VMEM((VR, TQ), F32),
        pltpu.VMEM((HB // 2, D), U32),
        pltpu.VMEM((8, D), F32),
        pltpu.VMEM((8, D), F32),
        pltpu.SemaphoreType.DMA((2 * NRB,)),
        pltpu.SemaphoreType.DMA((6,)),
        pltpu.SemaphoreType.DMA((S // OB,)),
    ]
    any_spec = pl.BlockSpec(memory_space=pl.ANY)
    out = pl.pallas_call(
        _kernel,
        out_shape=jax.ShapeDtypeStruct((S, D), A_x.dtype),
        in_specs=[any_spec] * 5,
        out_specs=any_spec,
        scratch_shapes=scratch,
        compiler_params=pltpu.CompilerParams(vmem_limit_bytes=100 * 1024 * 1024),
    )(x, A_wqkv, A_wo, B_wqkv, B_wo)
    return out.reshape(1, S, D)
```

```python
import math

import jax
import jax.numpy as jnp
import jax.experimental.pallas as pl
import jax.experimental.pallas.tpu as pltpu

S = 2048
D = 640
H = 32
DH = 20
LANES = 128
NDT = D // LANES
RB = 512
HB = 128
OB = 256
KG = 32
NRB = S // RB
TQ = 512
NQB = S // TQ
KC = 512
PKC = 128
LEAD = (1, 3, 4, 0)
NS = len(LEAD)
W = TQ // NS
NC = S // KC
VR = 24
UNROLL = 16
NPRE = 3
KVFIRST = 2
EPS = 1e-5
assert RB == TQ and RB == 2 * OB and KC == 4 * LANES

NT = (((1,), (1,)), ((), ()))

BF16 = jnp.bfloat16
F32 = jnp.float32
U32 = jnp.uint32
I32 = jnp.int32
I8 = jnp.int8

RND = 12582912.0


def _phi(t):
    return jnp.where(t > 0, t + 1.0, jnp.exp(t)) + 1e-6


def _layernorm(x):
    m = jnp.mean(x, axis=-1, keepdims=True)
    xc = x - m
    v = jnp.mean(xc * xc, axis=-1, keepdims=True)
    return xc * jax.lax.rsqrt(v + EPS)


def _kv_windows():
    wins = []
    for j in range(NDT):
        h0 = (j * LANES) // DH
        h1 = (j * LANES + LANES - 1) // DH
        lo = (h0 * DH) // 16 * 16
        hi = -(-((h1 + 1) * DH) // 16) * 16
        wins.append((lo, hi))
    return wins


WINS = _kv_windows()


def _iota(shape, dim):
    return jax.lax.broadcasted_iota(jnp.int32, shape, dim)


def _pack8(v):
    return pltpu.bitcast(v.astype(I8), U32)


def _limbs(t16):
    m = pltpu.bitcast(t16 + (RND + 8.0), I32)
    return m >> 4, (m + 56) >> 7, (m & 15) - 8


def _kernel(x_hbm, awqkv_hbm, awo_hbm, bwqkv_hbm, bwo_hbm, o_hbm,
            xio, awqkv, awo, bwqkv, bwo, awkt, bwqvt,
            x_scr, pq_scr, y_scr, g_scr, z_scr, mw_scr, zt_scr,
            xn_scr, kf_scr, ksc_scr,
            qw_scr, mg_scr, k8_scr, vt_scr, s_scr, ot_scr, mx_scr, mxc_scr, oacc_scr,
            pre_scr, kmax_scr, kinv_scr,
            xsem, wsem, osem):

    def piece(i, t):
        return pl.ds(pl.multiple_of(i * RB + t * HB, HB), HB)

    def piece2(i, t):
        return pl.ds(pl.multiple_of((i * RB + t * HB) // 2, HB // 2), HB // 2)

    def x_copy(i, first):
        if first:
            rows, sem = piece(i, 0), xsem.at[i]
        else:
            rows, sem = pl.ds(pl.multiple_of(i * RB + HB, HB), RB - HB), xsem.at[NRB + i]
        return pltpu.make_async_copy(x_hbm.at[rows, :], xio.at[rows, :], sem)

    def o_copy(n):
        rows = pl.ds(pl.multiple_of(n * OB, OB), OB)
        return pltpu.make_async_copy(xio.at[rows, :], o_hbm.at[rows, :], osem.at[n])

    cp_awk = pltpu.make_async_copy(awqkv_hbm.at[:, D:2 * D], awqkv.at[:, D:2 * D], wsem.at[0])
    cp_awq = pltpu.make_async_copy(awqkv_hbm.at[:, 0:D], awqkv.at[:, 0:D], wsem.at[1])
    cp_awv = pltpu.make_async_copy(awqkv_hbm.at[:, 2 * D:3 * D], awqkv.at[:, 2 * D:3 * D], wsem.at[2])
    cp_awo = pltpu.make_async_copy(awo_hbm, awo, wsem.at[3])
    cp_bwqkv = pltpu.make_async_copy(bwqkv_hbm, bwqkv, wsem.at[4])
    cp_bwo = pltpu.make_async_copy(bwo_hbm, bwo, wsem.at[5])

    def a_proj(i, xns):
        pkts = []
        for xn in xns:
            kt = jax.lax.dot_general(pltpu.bitcast(awkt[...], BF16), xn, NT,
                                     preferred_element_type=F32)
            pkts.append(_phi(kt))
        for t, xn in enumerate(xns):
            q = jnp.dot(xn, awqkv[:, 0:D], preferred_element_type=F32)
            pq_scr[piece2(i, t), :] = pltpu.bitcast(_phi(q).astype(BF16), U32)
        pkt = jnp.concatenate(pkts, axis=1)
        zacc = pkt[:, 0:LANES]
        for t in range(1, RB // LANES):
            zacc = zacc + pkt[:, t * LANES:(t + 1) * LANES]
        z_scr[...] += zacc
        g_scr[...] += jnp.dot(pkt.astype(BF16), jnp.concatenate(xns, axis=0),
                              preferred_element_type=F32)

    def a_y(i, t):
        pq = pltpu.bitcast(pq_scr[piece2(i, t), :], BF16)
        dent = jax.lax.dot_general(zt_scr[0:H, :], pq, NT, preferred_element_type=F32) + 1e-6
        rt = 1.0 / dent
        r = jnp.concatenate([rt] * (LANES // H), axis=0).T
        r_exp = jnp.concatenate(
            [jnp.take_along_axis(r, (_iota((HB, LANES), 1) + j * LANES) // DH, axis=1)
             for j in range(NDT)], axis=1)
        return (pq.astype(F32) * r_exp).astype(BF16)

    def a_norm(i):
        for t in range(NPRE):
            y_scr[t] = pltpu.bitcast(a_y(i, t), U32)

    def a_mid():
        kvs = []
        for j, (lo, hi) in enumerate(WINS):
            if j == KVFIRST:
                z = jnp.sum(z_scr[...].T, axis=0, keepdims=True)
                r0 = _iota((H, D), 0) * DH
                col = _iota((H, D), 1)
                zt_scr[0:H, :] = jnp.where((col >= r0) & (col < r0 + DH), z, 0.0).astype(BF16)
                a_norm(0)
            n = hi - lo
            kvj = jnp.dot(g_scr[lo:hi, :].astype(BF16),
                          awqkv[:, 2 * D + j * LANES:2 * D + (j + 1) * LANES],
                          preferred_element_type=F32)
            c0 = (_iota((1, LANES), 1) + j * LANES) // DH * DH - lo
            row = _iota((n, LANES), 0)
            kvs.append(jnp.where((row >= c0) & (row < c0 + DH), kvj, 0.0).astype(BF16))
        parts = [jnp.dot(kvs[j], awo[j * LANES:(j + 1) * LANES, :], preferred_element_type=F32)
                 for j in range(NDT)]
        for j, (lo, hi) in enumerate(WINS):
            s0 = lo if j == 0 else WINS[j - 1][1]
            s1 = hi if j == NDT - 1 else WINS[j + 1][0]
            mw_scr[s0 // 2:s1 // 2, :] = pltpu.bitcast(parts[j][s0 - lo:s1 - lo, :].astype(BF16), U32)
            if j < NDT - 1:
                mw_scr[s1 // 2:hi // 2, :] = pltpu.bitcast(
                    (parts[j][s1 - lo:hi - lo, :] + parts[j + 1][0:hi - s1, :]).astype(BF16), U32)
        kmax_scr[...] = jnp.zeros_like(kmax_scr)
        g_scr[...] = jnp.zeros_like(g_scr)
        z_scr[...] = jnp.zeros_like(z_scr)

    def a_out(y):
        return jnp.dot(y, pltpu.bitcast(mw_scr[...], BF16), preferred_element_type=F32)

    qscale = (DH ** -0.5) * math.log2(math.e)

    def b_proj_k(i, t, xn):
        k = jnp.dot(xn, bwqkv[:, D:2 * D], preferred_element_type=F32)
        kf_scr[piece(i, t), :] = k
        kmax_scr[...] = jnp.maximum(kmax_scr[...],
                                    jnp.max(jnp.abs(k).reshape(HB // 8, 8, D), axis=0))

    def b_scales():
        kmax = jnp.max(kmax_scr[...], axis=0, keepdims=True)
        kmax = jnp.maximum(kmax, 1e-30)
        kinv_scr[...] = jnp.broadcast_to((16.0 * 127.0) / kmax, (8, D))
        ksc_scr[...] = jnp.broadcast_to(kmax * (qscale / 127.0), (LANES, D)).T

    def b_proj_qv(i, t):
        cols = piece(i, t)
        lc = slice(t * HB, (t + 1) * HB)
        xn = pltpu.bitcast(xn_scr[piece2(i, t), :], BF16)
        qvt = jax.lax.dot_general(pltpu.bitcast(bwqvt[...], BF16), xn, NT,
                                  preferred_element_type=F32)
        row = _iota((VR, HB), 0)
        zero8 = jnp.zeros((8, HB), I32)
        for h in range(H):
            off = (h * DH) % 8
            w0 = h * DH - off
            q = jnp.where((row >= off) & (row < off + DH),
                          qvt[w0:w0 + VR, :] * ksc_scr[w0:w0 + VR, :], 0.0)
            qmax = jnp.max(jnp.abs(q), axis=0, keepdims=True) * (1.0 / 127.0)
            eb = jnp.clip(pltpu.bitcast(qmax, I32) >> 23, 66, 226)
            qa, q8, qf = _limbs(q * pltpu.bitcast((257 - eb) << 23, F32))
            pa = _pack8(jnp.concatenate([qa, zero8], axis=0))
            qw_scr[i * H + h, 0:8, lc] = pa
            qw_scr[i * H + h, 8:16, lc] = pa
            qw_scr[i * H + h, 16:24, lc] = _pack8(jnp.concatenate([q8, zero8], axis=0))
            qw_scr[i * H + h, 24:32, lc] = _pack8(jnp.concatenate([qf, zero8], axis=0))
            mg_scr[i * H + h, :, lc] = jnp.broadcast_to(((eb + 23) << 23) | 0x400000, (8, HB))
        sub = _iota((8, HB), 0)
        for p in range(H // 2):
            b = D + p * 2 * DH
            mid = qvt[b + 16:b + 24, :]
            vt_scr[2 * p, 0:16, cols] = qvt[b:b + 16, :]
            vt_scr[2 * p, 16:24, cols] = jnp.where(sub < 4, mid, 1.0)
            vt_scr[2 * p + 1, 0:8, cols] = jnp.where(sub < 4, 1.0, mid)
            vt_scr[2 * p + 1, 8:24, cols] = qvt[b + 24:b + 40, :]
        lane = _iota((KG // 4, LANES), 1)
        for n in range(HB // KG):
            r0 = i * RB + t * HB + n * KG
            kt = (kf_scr[pl.ds(pl.multiple_of(r0, KG), KG), :].reshape(KG // 8, 8, D)
                  * kinv_scr[...][None]).reshape(KG, D)
            ka, k8, kf = [_pack8(v) for v in _limbs(kt)]
            krows = pl.ds(pl.multiple_of(r0 // 4, KG // 4), KG // 4)
            for h in range(H):
                off = (h * DH) % 8
                g, a = divmod(h * DH, LANES)

                def place(l, r):
                    src = l[:, g * LANES:(g + 1) * LANES]
                    if a + DH > LANES:
                        src = jnp.where(lane >= LANES // 2, src,
                                        l[:, (g + 1) * LANES:(g + 2) * LANES])
                    shift = (32 * r + off - a) % LANES
                    return pltpu.roll(src, shift, 1) if shift else src

                lo = jnp.where(lane < 32, place(ka, 0), place(ka, 1))
                hi = jnp.where(lane < 96, place(kf, 2), place(k8, 3))
                k8_scr[h, krows, :] = jnp.where(lane < 64, lo, hi)

    def o_rows(i, t):
        cols = pl.ds(t * HB if isinstance(t, int) else pl.multiple_of(t * HB, HB), HB)
        return ot_scr[pl.ds(i * (H // 2), H // 2), :, cols].reshape(D, HB).T.astype(BF16)

    def b_attention():
        n_stage = NQB * H
        upc = KC // PKC
        ups = S // PKC
        ahead = [(upc - r) % upc for r in LEAD]

        def qk(i, slot, k0, k1, mx, p):
            ls = slice(p * W, (p + 1) * W)
            n = (k1 - k0) * PKC
            k = pltpu.bitcast(k8_scr[i & (H - 1), k0 * PKC // 4:k1 * PKC // 4, :], I8)
            q = pltpu.bitcast(qw_scr[i, :, ls], I8)
            acc = jnp.dot(k, q, preferred_element_type=I32)
            s = pltpu.bitcast(acc.reshape(n // 8, 8, W) + mg_scr[i, :, ls][None], F32)
            s_scr[slot, k0 * PKC:k1 * PKC, ls] = s.reshape(n, W)
            cm = jnp.max(s, axis=0)
            mx = cm if mx is None else jnp.maximum(mx, cm)
            if k1 == ups:
                mx_scr[slot, :, ls] = jnp.broadcast_to(jnp.max(mx, axis=0, keepdims=True), (8, W))
            return mx

        def pv(i, slot, c, o, p):
            ls = slice(p * W, (p + 1) * W)
            s = s_scr[slot, c * KC:(c + 1) * KC, ls].reshape(KC // 8, 8, W) - mx_scr[slot, :, ls][None]
            pt = jnp.exp2(s).reshape(KC, W)
            vt = vt_scr[i & (H - 1), :, c * KC:(c + 1) * KC]
            for sub in range(upc):
                ks = slice(sub * PKC, (sub + 1) * PKC)
                oc = jnp.dot(vt[:, ks], pt[ks, :], preferred_element_type=F32,
                             precision=jax.lax.Precision.DEFAULT)
                o = oc if o is None else o + oc
            if c == NC - 1:
                if slot == 1:
                    ot_scr[i >> 1, DH:2 * DH, ls] = o[4:VR, :] * (1.0 / o[0:1, :])
                else:
                    ot_scr[i >> 1, 0:DH, ls] = o[0:DH, :] * (1.0 / o[DH:DH + 1, :])
            return o

        mx = [None] * NS
        for c in range(NC):
            for p in range(NS):
                mx[p] = qk(0, 0, c * upc, (c + 1) * upc, mx[p], p)
        for p in range(NS):
            if ahead[p]:
                mxc_scr[:, p * W:(p + 1) * W] = qk(1, 1, 0, ahead[p], None, p)

        ops = []
        for p in range(NS):
            t, n, end = 0, ahead[p], ups * UNROLL + ahead[p]
            for b in range(-1, NC * UNROLL):
                if b >= 0:
                    ops.append((t, p, "pv", b - 1, None))
                    t += 102
                take = LEAD[p] if b < 0 else min(upc, end - n)
                if take:
                    ops.append((t, p, "qk", n, n + take))
                    t, n = t + 64 * take, n + take
        ops.sort(key=lambda op: op[:2])

        def body(j, carry):
            o = [oacc_scr[:, p * W:(p + 1) * W] for p in range(NS)]
            mx = [mxc_scr[:, p * W:(p + 1) * W] if ahead[p] else None for p in range(NS)]
            for _, p, kind, a, b in ops:
                if kind == "qk":
                    u = a // ups + 1
                    i = j * UNROLL + u
                    if u >= UNROLL:
                        i = jnp.minimum(i, n_stage - 1)
                    mx[p] = qk(i, u % 2, a % ups, (b - 1) % ups + 1, mx[p] if a % ups else None, p)
                else:
                    u, c = divmod(a, NC)
                    i = j * UNROLL + u if u >= 0 else jnp.maximum(j * UNROLL + u, 1)
                    o[p] = pv(i, u % 2, c, o[p] if c else None, p)
            for p in range(NS):
                oacc_scr[:, p * W:(p + 1) * W] = o[p]
                if ahead[p]:
                    mxc_scr[:, p * W:(p + 1) * W] = mx[p]
            return carry

        jax.lax.fori_loop(0, n_stage // UNROLL, body, 0)
        for p in range(NS):
            pv(n_stage - 1, 1, NC - 1, oacc_scr[:, p * W:(p + 1) * W], p)
        pre_scr[...] = pltpu.bitcast(o_rows(0, 0), U32)

    def b_out(i, t, first):
        o = pltpu.bitcast(pre_scr[...], BF16) if first else o_rows(i, t)
        return jnp.dot(o, bwo[...], preferred_element_type=F32)

    def residual_ln(i, t, out):
        x = x_scr[piece(i, t), :] + out
        x_scr[piece(i, t), :] = x
        return _layernorm(x).astype(BF16)

    def load_ln(i, t):
        x = xio[piece(i, t), :].astype(F32)
        x_scr[piece(i, t), :] = x
        return _layernorm(x).astype(BF16)

    x_copy(0, True).start()
    cp_awk.start()
    x_copy(0, False).start()
    cp_awq.start()
    x_copy(1, True).start()

    def zero_body(n, c):
        rows = pl.ds(pl.multiple_of(n * LANES, LANES), LANES)
        g_scr[rows, :] = jnp.zeros((LANES, D), F32)
        z_scr[rows, :] = jnp.zeros((LANES, LANES), F32)
        srows = pl.ds(pl.multiple_of(S - KC + jnp.minimum(n, 3) * LANES, LANES), LANES)
        s_scr[1, srows, :] = jnp.zeros((LANES, TQ), F32)
        return c

    jax.lax.fori_loop(0, NDT, zero_body, 0)
    mx_scr[1] = jnp.zeros((8, TQ), F32)
    oacc_scr[...] = jnp.zeros_like(oacc_scr)
    x_copy(0, True).wait()
    pre_scr[...] = pltpu.bitcast(load_ln(0, 0), U32)
    cp_awk.wait()
    awkt[...] = pltpu.bitcast(awqkv[:, D:2 * D].T, U32)
    cp_awq.wait()
    for i in range(1, NRB):
        x_copy(i, False).start()
        if i + 1 < NRB:
            x_copy(i + 1, True).start()
    cp_awv.start()
    cp_awo.start()
    cp_bwqkv.start()
    cp_bwo.start()

    def p1a(i, c):
        x_copy(i, False).wait()

        @pl.when(i + 1 < NRB)
        def _():
            x_copy(i + 1, True).wait()

        xns = [pltpu.bitcast(pre_scr[...], BF16)] + [load_ln(i, t) for t in range(1, RB // HB)]
        a_proj(i, xns)
        pre_scr[...] = pltpu.bitcast(load_ln(jnp.minimum(i + 1, NRB - 1), 0), U32)
        return c

    jax.lax.fori_loop(0, NRB, p1a, 0)

    cp_awv.wait()
    cp_awo.wait()
    cp_bwqkv.wait()
    cp_bwo.wait()

    def p2a(i, c):
        ys = [pltpu.bitcast(y_scr[t], BF16) if t < NPRE else a_y(i, t)
              for t in range(RB // HB)]
        xns = [residual_ln(i, t, a_out(ys[t])) for t in range(RB // HB)]
        a_norm(jnp.minimum(i + 1, NRB - 1))
        for t in range(RB // HB):
            xn_scr[piece2(i, t), :] = pltpu.bitcast(xns[t], U32)
            b_proj_k(i, t, xns[t])
        per = -(-2 * NDT // NRB)
        for n in range(per):
            tile = jnp.minimum(i * per + n, 2 * NDT - 1)
            c0 = pl.multiple_of(jnp.where(tile < NDT, tile, tile + NDT) * LANES, LANES)
            bwqvt[pl.ds(pl.multiple_of(tile * (LANES // 2), LANES // 2), LANES // 2), :] = pltpu.bitcast(
                bwqkv[:, pl.ds(c0, LANES)].T, U32)
        return c

    def p2b(i, c):
        b_scales()
        for t in range(RB // HB):
            b_proj_qv(i, t)
        return c

    def p1b(i, c):
        xns = [residual_ln(i, t, b_out(i, t, t == 0)) for t in range(RB // HB)]
        a_proj(i, xns)
        pre_scr[...] = pltpu.bitcast(o_rows(jnp.minimum(i + 1, NRB - 1), 0), U32)
        return c

    def p3(n, c):
        i = n >> 1
        for e in range(OB // HB):
            t = (n & 1) * (OB // HB) + e
            x = x_scr[piece(i, t), :] + b_out(i, t, e == 0)
            xio[piece(i, t), :] = x.astype(BF16)
        nn = jnp.minimum(n + 1, S // OB - 1)
        pre_scr[...] = pltpu.bitcast(o_rows(nn >> 1, (nn & 1) * (OB // HB)), U32)
        o_copy(n).start()
        return c

    def layer_pair(l, c):
        a_mid()
        jax.lax.fori_loop(0, NRB, p2a, 0)
        jax.lax.fori_loop(0, NRB, p2b, 0)
        b_attention()

        @pl.when(l == 0)
        def _():
            jax.lax.fori_loop(0, NRB, p1b, 0)

        @pl.when(l == 1)
        def _():
            jax.lax.fori_loop(0, S // OB, p3, 0)

        return c

    jax.lax.fori_loop(0, 2, layer_pair, 0)
    for n in range(S // OB):
        o_copy(n).wait()


@jax.jit
def pallas_interleave_layers__linear_attn_block__mha_block__prompt_kernel(
    A_x: jax.Array,
    A_wqkv: jax.Array,
    A_wo: jax.Array,
    B_x: jax.Array,
    B_wqkv: jax.Array,
    B_wo: jax.Array,
):
    del B_x
    x = A_x.reshape(S, D)

    scratch = [
        pltpu.VMEM((S, D), BF16),
        pltpu.VMEM((D, 3 * D), BF16),
        pltpu.VMEM((D, D), BF16),
        pltpu.VMEM((D, 3 * D), BF16),
        pltpu.VMEM((D, D), BF16),
        pltpu.VMEM((D // 2, D), U32),
        pltpu.VMEM((D, D), U32),
        pltpu.VMEM((S, D), F32),
        pltpu.VMEM((S // 2, D), U32),
        pltpu.VMEM((NPRE, HB // 2, D), U32),
        pltpu.VMEM((D, D), F32),
        pltpu.VMEM((D, LANES), F32),
        pltpu.VMEM((D // 2, D), U32),
        pltpu.VMEM((LANES, D), BF16),
        pltpu.VMEM((S // 2, D), U32),
        pltpu.VMEM((S, D), F32),
        pltpu.VMEM((D, LANES), F32),
        pltpu.VMEM((NQB * H, LANES // 4, TQ), U32),
        pltpu.VMEM((NQB * H, 8, TQ), I32),
        pltpu.VMEM((H, S // 4, LANES), U32),
        pltpu.VMEM((H, VR, S), F32),
        pltpu.VMEM((2, S, TQ), F32),
        pltpu.VMEM((NQB * H // 2, 2 * DH, TQ), F32),
        pltpu.VMEM((2, 8, TQ), F32),
        pltpu.VMEM((8, TQ), F32),
        pltpu.VMEM((VR, TQ), F32),
        pltpu.VMEM((HB // 2, D), U32),
        pltpu.VMEM((8, D), F32),
        pltpu.VMEM((8, D), F32),
        pltpu.SemaphoreType.DMA((2 * NRB,)),
        pltpu.SemaphoreType.DMA((6,)),
        pltpu.SemaphoreType.DMA((S // OB,)),
    ]
    any_spec = pl.BlockSpec(memory_space=pl.ANY)
    out = pl.pallas_call(
        _kernel,
        out_shape=jax.ShapeDtypeStruct((S, D), A_x.dtype),
        in_specs=[any_spec] * 5,
        out_specs=any_spec,
        scratch_shapes=scratch,
        compiler_params=pltpu.CompilerParams(vmem_limit_bytes=100 * 1024 * 1024),
    )(x, A_wqkv, A_wo, B_wqkv, B_wo)
    return out.reshape(1, S, D)
```
